```python
import jax
import jax.numpy as jnp

def _softmax(x, axis=-1):
    return jax.nn.softmax(x, axis=axis)
def _gelu(x):
    return jax.nn.gelu(x, approximate=True)
def _silu(x):
    return jax.nn.silu(x)
def _sigmoid(x):
    return jax.nn.sigmoid(x)
def _layernorm(x, axis=-1, eps=1e-5):
    m = jnp.mean(x, axis=axis, keepdims=True)
    v = jnp.var(x, axis=axis, keepdims=True)
    return (x - m) / jnp.sqrt(v + eps)
def _scatter_add(tgt, idx, src, axis=0):
    return tgt.at[idx].add(src)
def _segment_sum(src, seg, n):
    return jax.ops.segment_sum(src, seg, n)
class _Rng:
    def __init__(self, key):
        self._k = key
    def _next(self):
        self._k, sub = jax.random.split(self._k)
        return sub
    def normal(self, shape):
        return jax.random.normal(self._next(), shape, dtype=jnp.bfloat16)
    def randint(self, lo, hi, shape):
        return jax.random.randint(self._next(), shape, lo, hi, dtype=jnp.int32)
    def uniform(self, shape, lo=0.0, hi=1.0):
        return jax.random.uniform(self._next(), shape, jnp.bfloat16, lo, hi)
    def permutation(self, n):
        return jax.random.permutation(self._next(), n)


kernel_name = 'recurrent_scan__compressed_kv_cla__dense_activation_silu__decode'

def setup_inputs():
    _rng = _Rng(jax.random.key(int.from_bytes(__import__("os").urandom(4), "little")))
    _w = (lambda a: (lambda t: t.astype(jnp.bfloat16) if jnp.issubdtype(t.dtype, jnp.floating) else t)(jnp.asarray(a)))
    def _A_setup():
        B, H, Sq, Sk, D, M = 1, 32, 1, 32768, 128, 512
        Dc = 4 * D
        return {
            "x": _w((lambda *s: _rng.normal(s) * 0.05)(B, Sq, M)),
            "c_kv": _w((lambda *s: _rng.normal(s) * 0.05)(B, Sk, Dc)),
            "w_q": _w((lambda *s: _rng.normal(s) * 0.05)(M, H, D) * (M ** -0.5)),
            "w_uk": _w((lambda *s: _rng.normal(s) * 0.05)(Dc, H, D) * (Dc ** -0.5)),
            "w_uv": _w((lambda *s: _rng.normal(s) * 0.05)(Dc, H, D) * (Dc ** -0.5)),
            "w_o": _w((lambda *s: _rng.normal(s) * 0.05)(H, D, M) * ((H * D) ** -0.5)),
        }
    _A_in = _A_setup()

    def _B_setup():
        B, S, D, F = 1, 1, 512, 1376
        return {
            "x": _w((lambda *s: _rng.normal(s) * 0.05)(B, S, D)),
            "w1": _w((lambda *s: _rng.normal(s) * 0.05)(D, F) * (D ** -0.5)),
            "w2": _w((lambda *s: _rng.normal(s) * 0.05)(F, D) * (F ** -0.5)),
        }
    _B_in = _B_setup()

    return {
        "A_x": _A_in["x"],
        "A_c_kv": _A_in["c_kv"],
        "A_w_q": _A_in["w_q"],
        "A_w_uk": _A_in["w_uk"],
        "A_w_uv": _A_in["w_uv"],
        "A_w_o": _A_in["w_o"],
        "B_x": _B_in["x"],
        "B_w1": _B_in["w1"],
        "B_w2": _B_in["w2"],
    }

def reference(A_x, A_c_kv, A_w_q, A_w_uk, A_w_uv, A_w_o, B_x, B_w1, B_w2):
    def _A_ref(x, c_kv, w_q, w_uk, w_uv, w_o):
        B, Sq, M = x.shape[0], x.shape[1], x.shape[2]
        Sk = c_kv.shape[1]
        H, D = w_q.shape[1], w_q.shape[2]
        q = jnp.einsum("bqm,mhd->bhqd", x, w_q)
        k = jnp.einsum("bkc,chd->bhkd", c_kv, w_uk)
        v = jnp.einsum("bkc,chd->bhkd", c_kv, w_uv)
        scores = jnp.einsum("bhqd,bhkd->bhqk", q, k) * (D ** -0.5)
        off = Sk - Sq
        qi = jnp.arange(Sq)[:, None]
        kj = jnp.arange(Sk)[None, :]
        cmask = kj <= (qi + off)
        scores = jnp.where(cmask[None, None], scores, -1e9)
        p = _softmax(scores, axis=-1)
        ctx = jnp.einsum("bhqk,bhkd->bhqd", p, v)
        return jnp.einsum("bhqd,hdm->bqm", ctx, w_o)

    def _B_ref(x, w1, w2):
        h = jnp.einsum("bsd,df->bsf", x, w1)
        h = _silu(h)
        out = jnp.einsum("bsf,fd->bsd", h, w2)
        return out

    x = A_x
    xn = _layernorm(x, axis=-1)
    s = _A_ref(xn, A_c_kv, A_w_q, A_w_uk, A_w_uv, A_w_o)
    g = _silu(_B_ref(xn, B_w1, B_w2))
    return x + s * g
```

```python
import functools

import jax
import jax.numpy as jnp
from jax import lax
import jax.experimental.pallas as pl
import jax.experimental.pallas.tpu as pltpu

_F32 = jnp.float32
_BF16 = jnp.bfloat16
_LANES = 128

_KV_CHUNK = 4096
_WO_SPLITS = (24, 6, 2)


def _dot(a, b):
    return jnp.dot(a, b, preferred_element_type=_F32)


def _dot_nt(a, b):
    return lax.dot_general(a, b, (((1,), (1,)), ((), ())),
                           preferred_element_type=_F32)


def _silu(v):
    return v * jax.nn.sigmoid(v)


def _kernel(x_hbm, ckv_hbm, wq_hbm, wuk_hbm, wuv_hbm, wo_hbm, w1_hbm, w2_hbm,
            o_ref,
            x_v, ckv_v, wq_v, wuk_v, wuv_v, wo_v, w1_v, w2_v, e_v,
            sems, kv_sems, wo_sems, *, eps):
    n_c, n_h, n_d = wq_v.shape
    s_k = ckv_v.shape[0]
    n_kv = s_k // _KV_CHUNK
    n_j = n_c // _LANES
    kj = _LANES * n_h

    cp_x = pltpu.make_async_copy(x_hbm, x_v, sems.at[0])
    cp_wq = pltpu.make_async_copy(wq_hbm, wq_v, sems.at[1])
    cp_wuk = pltpu.make_async_copy(wuk_hbm, wuk_v, sems.at[2])
    cp_w1 = pltpu.make_async_copy(w1_hbm, w1_v, sems.at[3])
    cp_w2 = pltpu.make_async_copy(w2_hbm, w2_v, sems.at[4])
    cp_wuv = pltpu.make_async_copy(wuv_hbm, wuv_v, sems.at[5])

    def cp_kv(i):
        rows = pl.ds(pl.multiple_of(i * _KV_CHUNK, _KV_CHUNK), _KV_CHUNK)
        return pltpu.make_async_copy(ckv_hbm.at[0, rows, :], ckv_v.at[rows, :],
                                     kv_sems.at[i])

    wo_starts = [sum(_WO_SPLITS[:i]) for i in range(len(_WO_SPLITS))]

    def cp_wo(i):
        hs = pl.ds(wo_starts[i], _WO_SPLITS[i])
        return pltpu.make_async_copy(wo_hbm.at[hs], wo_v.at[hs], wo_sems.at[i])

    cp_x.start()
    cp_wq.start()
    cp_wuk.start()
    cp_w1.start()
    cp_w2.start()
    for i in range(n_kv):
        cp_kv(i).start()
    cp_wuv.start()
    for i in range(len(_WO_SPLITS)):
        cp_wo(i).start()

    e_row = lax.broadcasted_iota(jnp.int32, (_LANES, kj), 0)
    e_col = lax.broadcasted_iota(jnp.int32, (_LANES, kj), 1)
    e_v[...] = jnp.where(e_col // n_h == e_row, 1.0, 0.0).astype(_BF16)
    d_row = lax.broadcasted_iota(jnp.int32, (n_h, kj), 0)
    d_col = lax.broadcasted_iota(jnp.int32, (n_h, kj), 1)
    diag = (d_col % n_h) == d_row

    def expand(c_bf):
        stacked = jnp.concatenate(
            [c_bf[:, j * _LANES:(j + 1) * _LANES] for j in range(n_j)], axis=0)
        rep = _dot(stacked, e_v[...])
        return [jnp.where(diag, rep[j * n_h:(j + 1) * n_h], 0.0).astype(_BF16)
                for j in range(n_j)]

    def w_block(w_ref, j):
        return w_ref[j * _LANES:(j + 1) * _LANES].reshape(kj, n_d)

    def contract_major(xs, w_ref):
        out = _dot(xs[0], w_block(w_ref, 0))
        for j in range(1, n_j):
            out = out + _dot(xs[j], w_block(w_ref, j))
        return out

    cp_x.wait()
    x = x_v[0].astype(_F32)
    mu = jnp.mean(x, axis=-1, keepdims=True)
    xc = x - mu
    var = jnp.mean(xc * xc, axis=-1, keepdims=True)
    xn = (xc / jnp.sqrt(var + eps)).astype(_BF16)

    xs = expand(jnp.broadcast_to(xn, (n_h, n_c)))
    cp_wq.wait()
    q = contract_major(xs, wq_v).astype(_BF16)

    cp_wuk.wait()
    scale = n_d ** -0.5
    ts = []
    for j in range(n_j):
        t = _dot_nt(q, w_block(wuk_v, j))
        ts.append(jnp.where(diag, t * scale, 0.0).astype(_BF16))
    qa = _dot_nt(jnp.concatenate(ts, axis=0), e_v[...])
    q_abs = jnp.concatenate(
        [qa[j * n_h:(j + 1) * n_h] for j in range(n_j)], axis=1).astype(_BF16)

    cp_w1.wait()
    h1 = _silu(_dot_nt(xn, w1_v[...])).astype(_BF16)
    cp_w2.wait()
    g = _silu(_dot(h1, w2_v[...]))

    def kv_step(i, carry):
        m, l, acc = carry
        cp_kv(i).wait()
        rows = pl.ds(pl.multiple_of(i * _KV_CHUNK, _KV_CHUNK), _KV_CHUNK)
        kv = ckv_v[rows, :]
        s = _dot_nt(q_abs, kv)
        m_new = jnp.maximum(m, jnp.max(s, axis=1, keepdims=True))
        alpha = jnp.exp(m - m_new)
        p = jnp.exp(s - m_new)
        l = alpha * l + jnp.sum(p, axis=1, keepdims=True)
        acc = alpha * acc + _dot(p.astype(_BF16), kv)
        return m_new, l, acc

    m0 = jnp.full((n_h, 1), -jnp.inf, _F32)
    l0 = jnp.zeros((n_h, 1), _F32)
    a0 = jnp.zeros((n_h, n_c), _F32)
    _, l, acc = lax.fori_loop(0, n_kv, kv_step, (m0, l0, a0))
    ctx_c = (acc / l).astype(_BF16)

    xs = expand(ctx_c)
    cp_wuv.wait()
    ctx = contract_major(xs, wuv_v)

    sub = 8
    row = lax.broadcasted_iota(jnp.int32, (sub, n_d), 0)
    lhs = [jnp.where(row == h % sub,
                     ctx[(h // sub) * sub:(h // sub + 1) * sub], 0.0)
           for h in range(n_h)]
    s_acc = None
    for i, (h0, nh) in enumerate(zip(wo_starts, _WO_SPLITS)):
        a = jnp.concatenate(lhs[h0:h0 + nh], axis=1).astype(_BF16)
        cp_wo(i).wait()
        part = _dot(a, wo_v[h0:h0 + nh].reshape(nh * n_d, n_c))
        s_acc = part if s_acc is None else s_acc + part
    s = jnp.sum(s_acc, axis=0, keepdims=True)

    o_ref[0] = (x + s * g).astype(o_ref.dtype)


@jax.jit
def pallas_recurrent_scan__compressed_kv_cla__dense_activation_silu__decode_kernel(
    A_x: jax.Array,
    A_c_kv: jax.Array,
    A_w_q: jax.Array,
    A_w_uk: jax.Array,
    A_w_uv: jax.Array,
    A_w_o: jax.Array,
    B_x: jax.Array,
    B_w1: jax.Array,
    B_w2: jax.Array,
):
    del B_x
    b, s_q, m = A_x.shape
    _, s_k, d_c = A_c_kv.shape
    _, n_h, n_d = A_w_q.shape
    assert b == 1 and s_q == 1 and m == d_c and s_k % _KV_CHUNK == 0
    assert sum(_WO_SPLITS) == n_h

    w1_t = B_w1.T

    any_spec = pl.BlockSpec(memory_space=pl.ANY)
    return pl.pallas_call(
        functools.partial(_kernel, eps=1e-5),
        in_specs=[any_spec] * 8,
        out_specs=pl.BlockSpec(memory_space=pltpu.VMEM),
        out_shape=jax.ShapeDtypeStruct(A_x.shape, A_x.dtype),
        scratch_shapes=[
            pltpu.VMEM(A_x.shape, A_x.dtype),
            pltpu.VMEM((s_k, d_c), A_c_kv.dtype),
            pltpu.VMEM(A_w_q.shape, A_w_q.dtype),
            pltpu.VMEM(A_w_uk.shape, A_w_uk.dtype),
            pltpu.VMEM(A_w_uv.shape, A_w_uv.dtype),
            pltpu.VMEM(A_w_o.shape, A_w_o.dtype),
            pltpu.VMEM(w1_t.shape, w1_t.dtype),
            pltpu.VMEM(B_w2.shape, B_w2.dtype),
            pltpu.VMEM((_LANES, _LANES * n_h), _BF16),
            pltpu.SemaphoreType.DMA((6,)),
            pltpu.SemaphoreType.DMA((s_k // _KV_CHUNK,)),
            pltpu.SemaphoreType.DMA((len(_WO_SPLITS),)),
        ],
        compiler_params=pltpu.CompilerParams(
            vmem_limit_bytes=96 * 1024 * 1024),
    )(A_x, A_c_kv, A_w_q, A_w_uk, A_w_uv, A_w_o, w1_t, B_w2)
```

```python
import functools

import jax
import jax.numpy as jnp
from jax import lax
import jax.experimental.pallas as pl
import jax.experimental.pallas.tpu as pltpu

_F32 = jnp.float32
_BF16 = jnp.bfloat16
_LANES = 128

_PIECE_BYTES = 32 * 1024
_N_LANE = 8
_KV_BLOCK = 1024
_LOOK_A = 2
_LOOK_B = 4
_WO_TAIL = (4, 2, 2)


def _dot(a, b):
    return jnp.dot(a, b, preferred_element_type=_F32)


def _dot_nt(a, b):
    return lax.dot_general(a, b, (((1,), (1,)), ((), ())),
                           preferred_element_type=_F32)


def _silu(v):
    return v * jax.nn.sigmoid(v)


def _split(seq, n):
    q, r = divmod(len(seq), n)
    out, i = [], 0
    for k in range(n):
        m = q + (1 if k < r else 0)
        out.append(seq[i:i + m])
        i += m
    return out


def _round_robin(lanes):
    out = []
    for t in range(max(len(l) for l in lanes)):
        out.extend(l[t] for l in lanes if t < len(l))
    return out


def _kernel(x_hbm, ckv_hbm, wq_hbm, wuk_hbm, wuv_hbm, wo_hbm, w1_hbm, w2_hbm,
            o_ref,
            x_v, ckv_v, wq_v, wuk_v, wuv_v, wo_v, w1_v, w2_v, e_v, s_v,
            sems, *, eps):
    n_c, n_h, n_d = wq_v.shape
    n_blk = ckv_v.shape[0]
    s_k = n_blk * _KV_BLOCK
    n_j = n_c // _LANES
    kj = _LANES * n_h
    n_f = w1_v.shape[0]

    rows_pp = _PIECE_BYTES // (2 * n_c)
    slabs_pp = _PIECE_BYTES // (2 * n_h * n_d)
    lane_rows = _KV_BLOCK // _N_LANE
    rounds = lane_rows // rows_pp
    region = s_k // _N_LANE
    half = rounds * _N_LANE // 2

    S_X, S_WQ, S_WUK, S_W1, S_W2, S_WUV, S_WO = 0, 1, 2, 6, 7, 8, 9
    S_KV = S_WO + 1 + len(_WO_TAIL)

    def lead_pieces(src, dst, n, step, sem_of):
        return [(src.at[pl.ds(p * step, step)], dst.at[pl.ds(p * step, step)],
                 sem_of(p * step)) for p in range(n // step)]

    def kv_pieces(b, parity):
        out = []
        for r in range(rounds):
            for k in range(parity, _N_LANE, 2):
                src0 = k * region + r * rows_pp
                if isinstance(b, int):
                    st = src0 + b * lane_rows
                else:
                    st = pl.multiple_of(src0 + b * lane_rows, rows_pp)
                out.append((ckv_hbm.at[0, pl.ds(st, rows_pp), :],
                            ckv_v.at[b, pl.ds(k * lane_rows + r * rows_pp,
                                              rows_pp), :],
                            S_KV + b))
        return out

    def start(piece, prio):
        src, dst, s = piece
        pltpu.make_async_copy(src, dst, sems.at[s]).start(priority=prio)

    def wait(buf, s):
        pltpu.make_async_copy(buf, buf, sems.at[s]).wait()

    def start_pairs(a, b):
        for t in range(max(len(a), len(b))):
            if t < len(a):
                start(a[t], 0)
            if t < len(b):
                start(b[t], 1)

    wq_p = lead_pieces(wq_hbm, wq_v, n_c, slabs_pp, lambda c: S_WQ)
    wuk_p = lead_pieces(wuk_hbm, wuk_v, n_c, slabs_pp,
                        lambda c: S_WUK + c // _LANES)
    wuv_p = lead_pieces(wuv_hbm, wuv_v, n_c, slabs_pp, lambda c: S_WUV)
    w1_p = lead_pieces(w1_hbm, w1_v, n_f, rows_pp, lambda c: S_W1)
    w2_p = lead_pieces(w2_hbm, w2_v, n_f, rows_pp, lambda c: S_W2)
    hl = _N_LANE // 2
    g0 = _round_robin(_split(wq_p, hl) + _split(wuk_p, hl))
    g1 = _round_robin(_split(w1_p, hl) + _split(w2_p, hl))
    g2 = _round_robin(_split(wuv_p, _N_LANE))
    pre = g0 + g1 + g2
    assert len(g0) % 2 == 0 and len(g1) % 2 == 0 and len(g2) % 2 == 0
    pre_a, pre_b = pre[0::2], pre[1::2]
    for b in range(_LOOK_A):
        pre_a = pre_a + kv_pieces(b, 0)
    for b in range(_LOOK_B):
        pre_b = pre_b + kv_pieces(b, 1)
    prime = len(pre_b) - len(pre_a)

    n_head0 = n_h - sum(_WO_TAIL)
    wo_starts = [0, n_head0]
    for n in _WO_TAIL[:-1]:
        wo_starts.append(wo_starts[-1] + n)
    wo_sizes = [n_head0] + list(_WO_TAIL)

    def wo_sem(h):
        return S_WO + max(i for i, h0 in enumerate(wo_starts) if h >= h0)

    wo_p = [(wo_hbm.at[h, pl.ds(r * rows_pp, rows_pp), :],
             wo_v.at[h, pl.ds(r * rows_pp, rows_pp), :], wo_sem(h))
            for h in range(n_h) for r in range(n_d // rows_pp)]
    n0 = n_head0 * (n_d // rows_pp)
    wo_all = _round_robin(_split(wo_p[:n0], _N_LANE)) + wo_p[n0:]
    wo_a, wo_b = wo_all[0::2], wo_all[1::2]

    issued = [0]

    def issue_to(n_a):
        n_a = min(n_a, len(pre_a))
        lo = issued[0]
        if n_a > lo:
            start_pairs(pre_a[lo:n_a], pre_b[prime + lo:prime + n_a])
            issued[0] = n_a

    pltpu.make_async_copy(x_hbm, x_v, sems.at[S_X]).start(priority=0)
    for p in pre_b[:prime]:
        start(p, 1)
    issue_to(22)

    e_row = lax.broadcasted_iota(jnp.int32, (_LANES, kj), 0)
    e_col = lax.broadcasted_iota(jnp.int32, (_LANES, kj), 1)
    e_v[...] = jnp.where(e_col // n_h == e_row, 1.0, 0.0).astype(_BF16)
    d_row = lax.broadcasted_iota(jnp.int32, (n_h, kj), 0)
    d_col = lax.broadcasted_iota(jnp.int32, (n_h, kj), 1)
    diag = (d_col % n_h) == d_row

    def expand(c_bf):
        stacked = jnp.concatenate(
            [c_bf[:, j * _LANES:(j + 1) * _LANES] for j in range(n_j)], axis=0)
        rep = _dot(stacked, e_v[...])
        return [jnp.where(diag, rep[j * n_h:(j + 1) * n_h], 0.0).astype(_BF16)
                for j in range(n_j)]

    def w_block(w_ref, j):
        return w_ref[j * _LANES:(j + 1) * _LANES].reshape(kj, n_d)

    def contract_major(xs, w_ref):
        out = _dot(xs[0], w_block(w_ref, 0))
        for j in range(1, n_j):
            out = out + _dot(xs[j], w_block(w_ref, j))
        return out

    issue_to(26)
    wait(x_v, S_X)
    x = x_v[0].astype(_F32)
    mu = jnp.mean(x, axis=-1, keepdims=True)
    xc = x - mu
    var = jnp.mean(xc * xc, axis=-1, keepdims=True)
    xn = (xc / jnp.sqrt(var + eps)).astype(_BF16)

    xs = expand(jnp.broadcast_to(xn, (n_h, n_c)))
    ahead = 28
    ptr = len(g0) // 2 + ahead
    issue_to(ptr)
    wait(wq_v, S_WQ)
    q = contract_major(xs, wq_v).astype(_BF16)

    scale = n_d ** -0.5
    ts = []
    ptr += 10
    for j in range(n_j):
        issue_to(ptr)
        ptr += 5
        wait(wuk_v.at[pl.ds(j * _LANES, _LANES)], S_WUK + j)
        t = _dot_nt(q, w_block(wuk_v, j))
        ts.append(jnp.where(diag, t * scale, 0.0).astype(_BF16))
    issue_to(ptr)
    qa = _dot_nt(jnp.concatenate(ts, axis=0), e_v[...])
    q_abs = jnp.concatenate(
        [qa[j * n_h:(j + 1) * n_h] for j in range(n_j)], axis=1).astype(_BF16)

    ptr = max(ptr + 6, (len(g0) + len(g1)) // 2 + ahead)
    issue_to(ptr)
    wait(w1_v, S_W1)
    h1 = _silu(_dot_nt(xn, w1_v[...])).astype(_BF16)
    issue_to(ptr + 7)
    wait(w2_v, S_W2)
    g = _silu(_dot(h1, w2_v[...]))
    issue_to(len(pre_a))

    n_main = n_blk - _LOOK_B

    def kv_step(i, carry):
        m, l, acc = carry

        @pl.when(i < n_main)
        def _():
            start_pairs(kv_pieces(i + _LOOK_A, 0), kv_pieces(i + _LOOK_B, 1))

        for c in range(n_main, n_blk):
            @pl.when(i == c)
            def _(c=c):
                ba, bb = c + _LOOK_A, c + _LOOK_B
                a = (kv_pieces(ba, 0) if ba < n_blk else
                     wo_a[(ba - n_blk) * half:(ba - n_blk + 1) * half])
                b = wo_b[(bb - n_blk) * half:(bb - n_blk + 1) * half]
                start_pairs(a, b)

        wait(ckv_v.at[i], S_KV + i)
        kv = ckv_v[i]
        s = _dot_nt(q_abs, kv)
        m_new = jnp.maximum(m, jnp.max(s, axis=1, keepdims=True))
        alpha = jnp.exp(m - m_new)
        p = jnp.exp(s - m_new)
        l = alpha * l + jnp.sum(p, axis=1, keepdims=True)
        acc = alpha * acc + _dot(p.astype(_BF16), kv)
        return m_new, l, acc

    m0 = jnp.full((n_h, 1), -jnp.inf, _F32)
    l0 = jnp.zeros((n_h, 1), _F32)
    a0 = jnp.zeros((n_h, n_c), _F32)
    _, l, acc = lax.fori_loop(0, n_blk, kv_step, (m0, l0, a0))
    start_pairs(wo_a[_LOOK_A * half:], wo_b[_LOOK_B * half:])
    ctx_c = (acc / l).astype(_BF16)

    xs = expand(ctx_c)
    wait(wuv_v, S_WUV)
    ctx = contract_major(xs, wuv_v)

    sub = 8
    row = lax.broadcasted_iota(jnp.int32, (sub, n_d), 0)
    lhs = [jnp.where(row == h % sub,
                     ctx[(h // sub) * sub:(h // sub + 1) * sub], 0.0)
           for h in range(n_h)]
    n_wo = len(wo_sizes)
    for i, (h0, nh) in enumerate(zip(wo_starts, wo_sizes)):
        a = jnp.concatenate(lhs[h0:h0 + nh], axis=1).astype(_BF16)
        wait(wo_v.at[pl.ds(h0, nh)], S_WO + i)
        part = _dot(a, wo_v[h0:h0 + nh].reshape(nh * n_d, n_c))
        if i > 0:
            part = part + s_v[...]
        if i < n_wo - 1:
            s_v[...] = part
    s = jnp.sum(part, axis=0, keepdims=True)

    o_ref[0] = (x + s * g).astype(o_ref.dtype)


@jax.jit
def pallas_recurrent_scan__compressed_kv_cla__dense_activation_silu__decode_kernel(
    A_x: jax.Array,
    A_c_kv: jax.Array,
    A_w_q: jax.Array,
    A_w_uk: jax.Array,
    A_w_uv: jax.Array,
    A_w_o: jax.Array,
    B_x: jax.Array,
    B_w1: jax.Array,
    B_w2: jax.Array,
):
    del B_x
    b, s_q, m = A_x.shape
    _, s_k, d_c = A_c_kv.shape
    _, n_h, n_d = A_w_q.shape
    assert b == 1 and s_q == 1 and m == d_c and s_k % _KV_BLOCK == 0
    n_blk = s_k // _KV_BLOCK

    w1_t = B_w1.T

    any_spec = pl.BlockSpec(memory_space=pl.ANY)
    return pl.pallas_call(
        functools.partial(_kernel, eps=1e-5),
        in_specs=[any_spec] * 8,
        out_specs=pl.BlockSpec(memory_space=pltpu.VMEM),
        out_shape=jax.ShapeDtypeStruct(A_x.shape, A_x.dtype),
        scratch_shapes=[
            pltpu.VMEM(A_x.shape, A_x.dtype),
            pltpu.VMEM((n_blk, _KV_BLOCK, d_c), A_c_kv.dtype),
            pltpu.VMEM(A_w_q.shape, A_w_q.dtype),
            pltpu.VMEM(A_w_uk.shape, A_w_uk.dtype),
            pltpu.VMEM(A_w_uv.shape, A_w_uv.dtype),
            pltpu.VMEM(A_w_o.shape, A_w_o.dtype),
            pltpu.VMEM(w1_t.shape, w1_t.dtype),
            pltpu.VMEM(B_w2.shape, B_w2.dtype),
            pltpu.VMEM((_LANES, _LANES * n_h), _BF16),
            pltpu.VMEM((8, m), _F32),
            pltpu.SemaphoreType.DMA((10 + len(_WO_TAIL) + n_blk,)),
        ],
        compiler_params=pltpu.CompilerParams(
            vmem_limit_bytes=96 * 1024 * 1024,
            disable_bounds_checks=True,
            disable_semaphore_checks=True),
    )(A_x, A_c_kv, A_w_q, A_w_uk, A_w_uv, A_w_o, w1_t, B_w2)
```

```python
import functools

import jax
import jax.numpy as jnp
from jax import lax
import jax.experimental.pallas as pl
import jax.experimental.pallas.tpu as pltpu

_F32 = jnp.float32
_BF16 = jnp.bfloat16
_LANES = 128
_SUB = 8

_PIECE = 16
_SHIFT_A = 14
_SHIFT_B = 15
_N_LANE = 8
_KV_BLOCK = 1024
_LOOK_A = 2
_LOOK_B = 4


def _dot(a, b):
    return jnp.dot(a, b, preferred_element_type=_F32)


def _dot_nt(a, b):
    return lax.dot_general(a, b, (((1,), (1,)), ((), ())),
                           preferred_element_type=_F32)


def _silu(v):
    return v * jax.nn.sigmoid(v)


def _split(seq, n):
    q, r = divmod(len(seq), n)
    out, i = [], 0
    for k in range(n):
        m = q + (1 if k < r else 0)
        out.append(seq[i:i + m])
        i += m
    return out


def _round_robin(lanes):
    out = []
    for t in range(max(len(l) for l in lanes)):
        out.extend(l[t] for l in lanes if t < len(l))
    return out


def _cuts(lo, hi, shift):
    out = []
    while lo < hi:
        nxt = min(hi, lo + ((shift - lo - 1) % _PIECE) + 1)
        out.append((lo, nxt - lo))
        lo = nxt
    return out


def _tiles(a):
    r, c = a.shape
    a = a.reshape(r // _SUB, _SUB, c // _LANES, _LANES).transpose(0, 2, 1, 3)
    return a.reshape(-1, _SUB, _LANES)


def _untile(v, n_cb):
    v = v.reshape(-1, n_cb, _SUB, _LANES)
    return jnp.concatenate(
        [v[:, cb].reshape(-1, _LANES) for cb in range(n_cb)], axis=1)


_WO_GROUPS = (
    ((0, 1), 1, (0, 4), 4), ((0, 1), 0, (0, 4), 4),
    ((2,), 0, (0, 4), 4), ((3,), 0, (0, 4), 4), ((2,), 1, (0, 4), 4),
    ((3,), 1, (0, 2), 1), ((3,), 1, (2, 3), 1), ((3,), 1, (3, 4), 1),
)


def _kernel(x_hbm, ckv_hbm, wq_hbm, wuk_hbm, wuv_hbm, wo_hbm, w1_hbm, w2_hbm,
            o_ref,
            x_v, ckv_v, wq_v, wuk_v, wuv_v, wo_v, w1_v, w2_v, e_v, s_v,
            sems, *, eps, n_h):
    n_c = x_v.shape[-1]
    n_d = wq_v.shape[-1]
    n_j = n_c // _LANES
    kj = _LANES * n_h
    lane_tiles = ckv_v.shape[1]
    blk_tiles = _KV_BLOCK // _N_LANE // _SUB * n_j
    n_blk = lane_tiles // blk_tiles
    rounds = blk_tiles // _PIECE
    half = rounds * _N_LANE // 2
    head_tiles = n_d // _SUB * n_j

    S_X, S_WQ, S_WUK, S_W1, S_W2, S_WUV, S_KV0, S_WO = 0, 1, 2, 6, 7, 8, 9, 10
    S_KV = S_WO + len(_WO_GROUPS)

    def row_pieces(src, dst, shift, sem_of):
        return [(src.at[pl.ds(t * _SUB, n * _SUB)],
                 dst.at[pl.ds(t * _SUB, n * _SUB)], sem_of(t))
                for t, n in _cuts(0, src.shape[0] // _SUB, shift)]

    def tile_pieces(src, dst, shift, s):
        return [(src.at[pl.ds(t, n)], dst.at[pl.ds(t, n)], s)
                for t, n in _cuts(0, src.shape[0], shift)]

    def kv_pieces(b, parity):
        out = []
        for r in range(rounds):
            t = b * blk_tiles + _SHIFT_A + r * _PIECE
            n = _PIECE
            if isinstance(b, int):
                n = min(n, lane_tiles - t)
            if n > 0:
                out += [(ckv_hbm.at[k, pl.ds(t, n)], ckv_v.at[k, pl.ds(t, n)],
                         S_KV + b) for k in range(parity, _N_LANE, 2)]
        return out

    def start(piece, prio):
        src, dst, s = piece
        pltpu.make_async_copy(src, dst, sems.at[s]).start(priority=prio)

    def wait(buf, s):
        pltpu.make_async_copy(buf, buf, sems.at[s]).wait()

    def start_pairs(a, b):
        for t in range(max(len(a), len(b))):
            if t < len(a):
                start(a[t], 0)
            if t < len(b):
                start(b[t], 1)

    jt = kj // _SUB
    wq_p = row_pieces(wq_hbm, wq_v, _SHIFT_A, lambda t: S_WQ)
    wuk_p = row_pieces(wuk_hbm, wuk_v, _SHIFT_A, lambda t: S_WUK + t // jt)
    wuv_p = row_pieces(wuv_hbm, wuv_v, _SHIFT_A, lambda t: S_WUV)
    w1_p = tile_pieces(w1_hbm, w1_v, _SHIFT_B, S_W1)
    w2_p = tile_pieces(w2_hbm, w2_v, _SHIFT_B, S_W2)
    kv0_p = [(ckv_hbm.at[k, pl.ds(0, _SHIFT_A)], ckv_v.at[k, pl.ds(0, _SHIFT_A)],
              S_KV0) for k in range(_N_LANE)]
    g0 = _round_robin(_split(wq_p, 4) + _split(wuk_p, 4))
    l1, l2, lv = _split(w1_p, 2), _split(w2_p, 2), _split(wuv_p, 4)
    g1 = _round_robin([l1[0], lv[0], lv[1], l2[0], l1[1], lv[2], lv[3], l2[1]])
    n_ffn = 8 * max(len(l) for l in l1 + l2)
    pre = g0 + g1 + kv0_p
    pre_a, pre_b = pre[1::2], pre[0::2]
    for b in range(_LOOK_A):
        pre_a = pre_a + kv_pieces(b, 0)
    for b in range(_LOOK_B):
        pre_b = pre_b + kv_pieces(b, 1)
    prime = len(pre_b) - len(pre_a)

    wo_lane_tiles = wo_v.shape[2]
    wo_a, wo_b, wo_rng = [], [], []
    for gi, (qs, prio, (p0, p1), rr) in enumerate(_WO_GROUPS):
        lo = qs[0] * head_tiles + (_SHIFT_A if qs[0] else 0)
        hi = min((qs[-1] + 1) * head_tiles + _SHIFT_A, wo_lane_tiles)
        lanes = [[(wo_hbm.at[p, prio, pl.ds(t, n)], wo_v.at[p, prio, pl.ds(t, n)],
                   S_WO + gi) for t, n in _cuts(lo, hi, _SHIFT_A)]
                 for p in range(p0, p1)]
        ps = [x for t in range(0, len(lanes), rr)
              for x in _round_robin(lanes[t:t + rr])]
        (wo_b if prio else wo_a).extend(ps)
        wo_rng.append((lo, hi))
    wo_a, wo_b = _split(wo_a, 4), _split(wo_b, 4)

    issued = [0]

    def issue_to(n_a):
        n_a = min(n_a, len(pre_a))
        lo = issued[0]
        if n_a > lo:
            start_pairs(pre_a[lo:n_a], pre_b[prime + lo:prime + n_a])
            issued[0] = n_a

    pltpu.make_async_copy(x_hbm, x_v, sems.at[S_X]).start(priority=0)
    for p in pre_b[:prime]:
        start(p, 1)
    issue_to(22)

    e_row = lax.broadcasted_iota(jnp.int32, (_LANES, kj), 0)
    e_col = lax.broadcasted_iota(jnp.int32, (_LANES, kj), 1)
    e_v[...] = jnp.where(e_col // n_h == e_row, 1.0, 0.0).astype(_BF16)
    d_row = lax.broadcasted_iota(jnp.int32, (n_h, kj), 0)
    d_col = lax.broadcasted_iota(jnp.int32, (n_h, kj), 1)
    diag = (d_col % n_h) == d_row

    def expand(c_bf):
        stacked = jnp.concatenate(
            [c_bf[:, j * _LANES:(j + 1) * _LANES] for j in range(n_j)], axis=0)
        rep = _dot(stacked, e_v[...])
        return [jnp.where(diag, rep[j * n_h:(j + 1) * n_h], 0.0).astype(_BF16)
                for j in range(n_j)]

    def w_block(w_ref, j):
        return w_ref[j * kj:(j + 1) * kj]

    def contract_major(xs, w_ref):
        out = _dot(xs[0], w_block(w_ref, 0))
        for j in range(1, n_j):
            out = out + _dot(xs[j], w_block(w_ref, j))
        return out

    issue_to(26)
    wait(x_v, S_X)
    x = x_v[0].astype(_F32)
    mu = jnp.mean(x, axis=-1, keepdims=True)
    xc = x - mu
    var = jnp.mean(xc * xc, axis=-1, keepdims=True)
    xn = (xc / jnp.sqrt(var + eps)).astype(_BF16)

    xs = expand(jnp.broadcast_to(xn, (n_h, n_c)))
    ahead = 30
    ptr = len(g0) // 2 + ahead
    issue_to(ptr)
    wait(wq_v, S_WQ)
    q = contract_major(xs, wq_v).astype(_BF16)

    scale = n_d ** -0.5
    ts = []
    ptr += 10
    for j in range(n_j):
        issue_to(ptr)
        ptr += 6
        lo = j * jt + (_SHIFT_A if j else 0)
        hi = min((j + 1) * jt + _SHIFT_A, n_j * jt)
        wait(wuk_v.at[pl.ds(lo * _SUB, (hi - lo) * _SUB)], S_WUK + j)
        t = _dot_nt(q, w_block(wuk_v, j))
        ts.append(jnp.where(diag, t * scale, 0.0).astype(_BF16))
    issue_to(ptr)
    qa = _dot_nt(jnp.concatenate(ts, axis=0), e_v[...])
    q_abs = jnp.concatenate(
        [qa[j * n_h:(j + 1) * n_h] for j in range(n_j)], axis=1).astype(_BF16)

    ptr = max(ptr + 10, (len(g0) + n_ffn) // 2 + ahead)
    issue_to(ptr)
    wait(w1_v, S_W1)
    h1 = _silu(_dot_nt(xn, _untile(w1_v[...], n_j))).astype(_BF16)
    issue_to(ptr + 7)
    wait(w2_v, S_W2)
    g = _silu(_dot(h1, _untile(w2_v[...], n_j)))
    issue_to(len(pre_a))
    wait(ckv_v.at[:, pl.ds(0, _SHIFT_A)], S_KV0)

    n_main = n_blk - _LOOK_B - 1

    def kv_step(i, carry):
        m, l, acc = carry

        @pl.when(i < n_main)
        def _():
            start_pairs(kv_pieces(i + _LOOK_A, 0), kv_pieces(i + _LOOK_B, 1))

        for c in range(n_main, n_blk):
            @pl.when(i == c)
            def _(c=c):
                ba, bb = c + _LOOK_A, c + _LOOK_B
                a = kv_pieces(ba, 0) if ba < n_blk else wo_a[ba - n_blk]
                b = kv_pieces(bb, 1) if bb < n_blk else wo_b[bb - n_blk]
                start_pairs(a, b)

        t0 = i * blk_tiles

        @pl.when(i < n_blk - 1)
        def _():
            wait(ckv_v.at[:, pl.ds(t0 + _SHIFT_A, blk_tiles)], S_KV + i)

        @pl.when(i == n_blk - 1)
        def _():
            wait(ckv_v.at[:, pl.ds(lane_tiles - blk_tiles + _SHIFT_A,
                                   blk_tiles - _SHIFT_A)], S_KV + n_blk - 1)

        kv = _untile(ckv_v[:, pl.ds(t0, blk_tiles)], n_j)
        s = _dot_nt(q_abs, kv)
        m_new = jnp.maximum(m, jnp.max(s, axis=1, keepdims=True))
        alpha = jnp.exp(m - m_new)
        p = jnp.exp(s - m_new)
        l = alpha * l + jnp.sum(p, axis=1, keepdims=True)
        acc = alpha * acc + _dot(p.astype(_BF16), kv)
        return m_new, l, acc

    m0 = jnp.full((n_h, 1), -jnp.inf, _F32)
    l0 = jnp.zeros((n_h, 1), _F32)
    a0 = jnp.zeros((n_h, n_c), _F32)
    _, l, acc = lax.fori_loop(0, n_blk, kv_step, (m0, l0, a0))
    start_pairs(sum(wo_a[_LOOK_A:], []), sum(wo_b[_LOOK_B:], []))
    ctx_c = (acc / l).astype(_BF16)

    xs = expand(ctx_c)
    wait(wuv_v, S_WUV)
    ctx = contract_major(xs, wuv_v)

    sub = 8
    row = lax.broadcasted_iota(jnp.int32, (sub, n_d), 0)
    lhs = [jnp.where(row == h % sub,
                     ctx[(h // sub) * sub:(h // sub + 1) * sub], 0.0)
           for h in range(n_h)]
    per = n_h // _N_LANE
    n_wo = len(_WO_GROUPS)
    for i, (qs, prio, (p0, p1), _) in enumerate(_WO_GROUPS):
        heads = [(2 * p + prio) * per + qq for p in range(p0, p1) for qq in qs]
        a = jnp.concatenate([lhs[h] for h in heads], axis=1).astype(_BF16)
        lo, hi = wo_rng[i]
        wait(wo_v.at[pl.ds(p0, p1 - p0), prio, pl.ds(lo, hi - lo)], S_WO + i)
        w = wo_v[p0:p1, prio,
                 qs[0] * head_tiles:(qs[-1] + 1) * head_tiles]
        part = _dot(a, _untile(w, n_j))
        if i > 0:
            part = part + s_v[...]
        if i < n_wo - 1:
            s_v[...] = part
    s = jnp.sum(part, axis=0, keepdims=True)

    o_ref[0] = (x + s * g).astype(o_ref.dtype)


@jax.jit
def pallas_recurrent_scan__compressed_kv_cla__dense_activation_silu__decode_kernel(
    A_x: jax.Array,
    A_c_kv: jax.Array,
    A_w_q: jax.Array,
    A_w_uk: jax.Array,
    A_w_uv: jax.Array,
    A_w_o: jax.Array,
    B_x: jax.Array,
    B_w1: jax.Array,
    B_w2: jax.Array,
):
    del B_x
    b, s_q, m = A_x.shape
    _, s_k, d_c = A_c_kv.shape
    _, n_h, n_d = A_w_q.shape
    assert b == 1 and s_q == 1 and m == d_c and s_k % _KV_BLOCK == 0
    n_blk = s_k // _KV_BLOCK

    ckv = _tiles(A_c_kv[0]).reshape(_N_LANE, -1, _SUB, _LANES)
    wq, wuk, wuv = (w.reshape(-1, n_d) for w in (A_w_q, A_w_uk, A_w_uv))
    wo = _tiles(A_w_o.reshape(-1, m)).reshape(_N_LANE // 2, 2, -1, _SUB, _LANES)
    w1 = _tiles(B_w1.T)
    w2 = _tiles(B_w2)
    ops = (A_x, ckv, wq, wuk, wuv, wo, w1, w2)

    return pl.pallas_call(
        functools.partial(_kernel, eps=1e-5, n_h=n_h),
        in_specs=[pl.BlockSpec(memory_space=pl.ANY)] * len(ops),
        out_specs=pl.BlockSpec(memory_space=pltpu.VMEM),
        out_shape=jax.ShapeDtypeStruct(A_x.shape, A_x.dtype),
        scratch_shapes=[pltpu.VMEM(a.shape, a.dtype) for a in ops] + [
            pltpu.VMEM((_LANES, _LANES * n_h), _BF16),
            pltpu.VMEM((8, m), _F32),
            pltpu.SemaphoreType.DMA((10 + len(_WO_GROUPS) + n_blk,)),
        ],
        compiler_params=pltpu.CompilerParams(
            vmem_limit_bytes=96 * 1024 * 1024,
            disable_bounds_checks=True,
            disable_semaphore_checks=True),
    )(*ops)
```

```python
import functools

import jax
import jax.numpy as jnp
from jax import lax
import jax.experimental.pallas as pl
import jax.experimental.pallas.tpu as pltpu

_F32 = jnp.float32
_BF16 = jnp.bfloat16
_LANES = 128
_SUB = 8

_PIECE = 16
_SHIFT_A = 14
_SHIFT_B = 15
_N_LANE = 8
_KV_BLOCK = 1024
_LOOK_A = 2
_LOOK_B = 4


def _dot(a, b):
    return jnp.dot(a, b, preferred_element_type=_F32)


def _dot_nt(a, b):
    return lax.dot_general(a, b, (((1,), (1,)), ((), ())),
                           preferred_element_type=_F32)


def _silu(v):
    return v * jax.nn.sigmoid(v)


def _split(seq, n):
    q, r = divmod(len(seq), n)
    out, i = [], 0
    for k in range(n):
        m = q + (1 if k < r else 0)
        out.append(seq[i:i + m])
        i += m
    return out


def _round_robin(lanes):
    out = []
    for t in range(max(len(l) for l in lanes)):
        out.extend(l[t] for l in lanes if t < len(l))
    return out


def _tree_sum(xs):
    while len(xs) > 1:
        xs = [xs[i] + xs[i + 1] if i + 1 < len(xs) else xs[i]
              for i in range(0, len(xs), 2)]
    return xs[0]


def _cuts(lo, hi, shift):
    out = []
    while lo < hi:
        nxt = min(hi, lo + ((shift - lo - 1) % _PIECE) + 1)
        out.append((lo, nxt - lo))
        lo = nxt
    return out


def _tiles(a):
    r, c = a.shape
    a = a.reshape(r // _SUB, _SUB, c // _LANES, _LANES).transpose(0, 2, 1, 3)
    return a.reshape(-1, _SUB, _LANES)


def _untile(v, n_cb):
    v = v.reshape(-1, n_cb, _SUB, _LANES)
    return jnp.concatenate(
        [v[:, cb].reshape(-1, _LANES) for cb in range(n_cb)], axis=1)


_WO_MXU = (((0, 1), 1), ((0, 1), 0), ((2,), 0), ((3,), 0), ((2,), 1))
_N_WO_VPU = 5
_KV_ORDER = ((0, 4, 2, 6), (1, 5, 3, 7))


def _kernel(x_hbm, ckv_hbm, wq_hbm, wuk_hbm, wuv_hbm, wo_hbm, w1_hbm, w2_hbm,
            o_ref,
            x_v, ckv_v, wq_v, wuk_v, wuv_v, wo_v, w1_v, w2_v, e_v, s_v,
            sems, *, eps, n_h):
    n_c = x_v.shape[-1]
    n_d = wq_v.shape[-1]
    n_j = n_c // _LANES
    kj = _LANES * n_h
    lane_tiles = ckv_v.shape[1]
    blk_tiles = _KV_BLOCK // _N_LANE // _SUB * n_j
    n_blk = lane_tiles // blk_tiles
    rounds = blk_tiles // _PIECE
    half = rounds * _N_LANE // 2
    head_tiles = n_d // _SUB * n_j

    S_X, S_WQ, S_WUK, S_W1, S_W2, S_WUV, S_KV0, S_WO = 0, 1, 2, 6, 7, 8, 9, 10
    S_KV = S_WO + len(_WO_MXU) + _N_WO_VPU

    def row_pieces(src, dst, shift, sem_of):
        return [(src.at[pl.ds(t * _SUB, n * _SUB)],
                 dst.at[pl.ds(t * _SUB, n * _SUB)], sem_of(t))
                for t, n in _cuts(0, src.shape[0] // _SUB, shift)]

    def tile_pieces(src, dst, shift, s):
        return [(src.at[pl.ds(t, n)], dst.at[pl.ds(t, n)], s)
                for t, n in _cuts(0, src.shape[0], shift)]

    def kv_pieces(b, parity):
        out = []
        for r in range(rounds):
            t = b * blk_tiles + _SHIFT_A + r * _PIECE
            n = _PIECE
            if isinstance(b, int):
                n = min(n, lane_tiles - t)
            if n > 0:
                out += [(ckv_hbm.at[k, pl.ds(t, n)], ckv_v.at[k, pl.ds(t, n)],
                         S_KV + b) for k in _KV_ORDER[parity]]
        return out

    def start(piece, prio):
        src, dst, s = piece
        pltpu.make_async_copy(src, dst, sems.at[s]).start(priority=prio)

    def wait(buf, s):
        pltpu.make_async_copy(buf, buf, sems.at[s]).wait()

    def start_pairs(a, b):
        for t in range(max(len(a), len(b))):
            if t < len(a):
                start(a[t], 0)
            if t < len(b):
                start(b[t], 1)

    jt = kj // _SUB
    wq_p = row_pieces(wq_hbm, wq_v, _SHIFT_A, lambda t: S_WQ)
    wuk_p = row_pieces(wuk_hbm, wuk_v, _SHIFT_A, lambda t: S_WUK + t // jt)
    wuv_p = row_pieces(wuv_hbm, wuv_v, _SHIFT_A, lambda t: S_WUV)
    w1_p = tile_pieces(w1_hbm, w1_v, _SHIFT_B, S_W1)
    w2_p = tile_pieces(w2_hbm, w2_v, _SHIFT_B, S_W2)
    kv0_p = [(ckv_hbm.at[k, pl.ds(0, _SHIFT_A)], ckv_v.at[k, pl.ds(0, _SHIFT_A)],
              S_KV0) for k in range(_N_LANE)]
    g0 = _round_robin(_split(wq_p, 4) + _split(wuk_p, 4))
    l1, l2, lv = _split(w1_p, 2), _split(w2_p, 2), _split(wuv_p, 4)
    g1 = _round_robin([l1[0], lv[0], lv[1], l2[0], l1[1], lv[2], lv[3], l2[1]])
    n_ffn = 8 * max(len(l) for l in l1 + l2)
    pre = g0 + g1 + kv0_p
    pre_a, pre_b = pre[1::2], pre[0::2]
    for b in range(_LOOK_A):
        pre_a = pre_a + kv_pieces(b, 0)
    for b in range(_LOOK_B):
        pre_b = pre_b + kv_pieces(b, 1)
    prime = len(pre_b) - len(pre_a)

    wo_lane_tiles = wo_v.shape[2]
    n_pair = _N_LANE // 2

    def wo_pieces(p, prio, lo, hi, s):
        return [(wo_hbm.at[p, prio, pl.ds(t, n)], wo_v.at[p, prio, pl.ds(t, n)],
                 s) for t, n in _cuts(lo, hi, _SHIFT_A)]

    wo_a, wo_b, wo_rng = [], [], []
    for gi, (qs, prio) in enumerate(_WO_MXU):
        lo = qs[0] * head_tiles + (_SHIFT_A if qs[0] else 0)
        hi = min((qs[-1] + 1) * head_tiles + _SHIFT_A, wo_lane_tiles)
        (wo_b if prio else wo_a).extend(_round_robin(
            [wo_pieces(p, prio, lo, hi, S_WO + gi) for p in range(n_pair)]))
        wo_rng.append((lo, hi))
    q3 = wo_lane_tiles - head_tiles
    cut = q3 + _SHIFT_A + 2 * _PIECE
    wo_vpu = [(p, q3 + _SHIFT_A, q3, wo_lane_tiles) for p in range(n_pair - 1)]
    wo_vpu += [(n_pair - 1, q3 + _SHIFT_A, q3, cut),
               (n_pair - 1, cut, cut, wo_lane_tiles)]
    assert len(wo_vpu) == _N_WO_VPU
    for gi, (p, lo, _, hi) in enumerate(wo_vpu):
        wo_b.extend(wo_pieces(p, 1, lo, hi, S_WO + len(_WO_MXU) + gi))
    wo_a, wo_b = _split(wo_a, 4), _split(wo_b, 4)

    issued = [0]

    def issue_to(n_a):
        n_a = min(n_a, len(pre_a))
        lo = issued[0]
        if n_a > lo:
            start_pairs(pre_a[lo:n_a], pre_b[prime + lo:prime + n_a])
            issued[0] = n_a

    pltpu.make_async_copy(x_hbm, x_v, sems.at[S_X]).start(priority=0)
    for p in pre_b[:prime]:
        start(p, 1)
    issue_to(22)

    e_row = lax.broadcasted_iota(jnp.int32, (_LANES, kj), 0)
    e_col = lax.broadcasted_iota(jnp.int32, (_LANES, kj), 1)
    e_v[...] = jnp.where(e_col // n_h == e_row, 1.0, 0.0).astype(_BF16)
    d_row = lax.broadcasted_iota(jnp.int32, (n_h, kj), 0)
    d_col = lax.broadcasted_iota(jnp.int32, (n_h, kj), 1)
    diag = (d_col % n_h) == d_row

    def w_block(w_ref, j):
        return w_ref[j * kj:(j + 1) * kj]

    n_a = _LANES // n_h
    diag1 = diag[:, :_LANES]

    def contract_major(c, w_ref):
        out = None
        for j in range(n_j):
            cj = pltpu.roll(c[:, j * _LANES:(j + 1) * _LANES], 0, 1,
                            stride=1, stride_axis=0).astype(_BF16)
            x = jnp.concatenate(
                [jnp.where(diag1, pltpu.roll(cj, (_LANES - r) % _LANES, 1),
                           jnp.zeros_like(cj)) for r in range(n_h)], axis=1)
            w = w_block(w_ref, j).reshape(n_a, n_h, n_h, n_d)
            w = jnp.swapaxes(w, 0, 1).reshape(kj, n_d)
            part = _dot(x, w)
            out = part if out is None else out + part
        return out

    issue_to(26)
    wait(x_v, S_X)
    x = x_v[0].astype(_F32)
    mu = jnp.mean(x, axis=-1, keepdims=True)
    xc = x - mu
    var = jnp.mean(xc * xc, axis=-1, keepdims=True)
    xn = (xc / jnp.sqrt(var + eps)).astype(_BF16)

    ahead = 30
    ptr = len(g0) // 2 + ahead
    issue_to(ptr)
    wait(wq_v, S_WQ)
    q = contract_major(jnp.broadcast_to(xn.astype(_F32), (n_h, n_c)),
                       wq_v).astype(_BF16)

    scale = n_d ** -0.5
    ts = []
    ptr += 10
    for j in range(n_j):
        issue_to(ptr)
        ptr += 6
        lo = j * jt + (_SHIFT_A if j else 0)
        hi = min((j + 1) * jt + _SHIFT_A, n_j * jt)
        wait(wuk_v.at[pl.ds(lo * _SUB, (hi - lo) * _SUB)], S_WUK + j)
        t = _dot_nt(q, w_block(wuk_v, j))
        ts.append(jnp.where(diag, t * scale, 0.0).astype(_BF16))
    issue_to(ptr)
    qa = _dot_nt(jnp.concatenate(ts, axis=0), e_v[...])
    q_abs = jnp.concatenate(
        [qa[j * n_h:(j + 1) * n_h] for j in range(n_j)], axis=1).astype(_BF16)

    ptr = max(ptr + 10, (len(g0) + n_ffn) // 2 + ahead)
    issue_to(ptr)
    wait(w1_v, S_W1)
    h1 = _silu(_dot_nt(xn, _untile(w1_v[...], n_j))).astype(_BF16)
    issue_to(ptr + 7)
    wait(w2_v, S_W2)
    g = _silu(_dot(h1, _untile(w2_v[...], n_j)))
    issue_to(len(pre_a))
    wait(ckv_v.at[:, pl.ds(0, _SHIFT_A)], S_KV0)

    n_main = n_blk - _LOOK_B - 1

    def kv_step(i, carry):
        m, l, acc = carry

        @pl.when(i < n_main)
        def _():
            start_pairs(kv_pieces(i + _LOOK_A, 0), kv_pieces(i + _LOOK_B, 1))

        for c in range(n_main, n_blk):
            @pl.when(i == c)
            def _(c=c):
                ba, bb = c + _LOOK_A, c + _LOOK_B
                a = kv_pieces(ba, 0) if ba < n_blk else wo_a[ba - n_blk]
                b = kv_pieces(bb, 1) if bb < n_blk else wo_b[bb - n_blk]
                start_pairs(a, b)

        t0 = i * blk_tiles

        @pl.when(i < n_blk - 1)
        def _():
            wait(ckv_v.at[:, pl.ds(t0 + _SHIFT_A, blk_tiles)], S_KV + i)

        @pl.when(i == n_blk - 1)
        def _():
            wait(ckv_v.at[:, pl.ds(lane_tiles - blk_tiles + _SHIFT_A,
                                   blk_tiles - _SHIFT_A)], S_KV + n_blk - 1)

        kv = _untile(ckv_v[:, pl.ds(t0, blk_tiles)], n_j)
        s = _dot_nt(q_abs, kv)
        m_new = jnp.maximum(m, jnp.max(s, axis=1, keepdims=True))
        alpha = jnp.exp(m - m_new)
        p = jnp.exp(s - m_new)
        l = alpha * l + jnp.sum(p, axis=1, keepdims=True)
        acc = alpha * acc + _dot(p.astype(_BF16), kv)
        return m_new, l, acc

    m0 = jnp.full((n_h, 1), -jnp.inf, _F32)
    l0 = jnp.zeros((n_h, 1), _F32)
    a0 = jnp.zeros((n_h, n_c), _F32)
    _, l, acc = lax.fori_loop(0, n_blk, kv_step, (m0, l0, a0))
    start_pairs(wo_a[2], [])
    ctx_c = acc / l

    wait(wuv_v, S_WUV)
    ctx = contract_major(ctx_c, wuv_v)
    start_pairs(wo_a[3], [])

    sub = 8
    row = lax.broadcasted_iota(jnp.int32, (sub, n_d), 0)
    lhs = [jnp.where(row == h % sub,
                     ctx[(h // sub) * sub:(h // sub + 1) * sub], 0.0)
           for h in range(n_h)]
    per = n_h // _N_LANE
    ctx_r = ctx.astype(_BF16).astype(_F32)
    col = [jnp.transpose(jnp.broadcast_to(
        ctx_r[(2 * p + 2) * per - 1:(2 * p + 2) * per], (n_d, n_d)))
        for p in range(n_pair)]
    for i, (qs, prio) in enumerate(_WO_MXU):
        heads = [(2 * p + prio) * per + qq for p in range(n_pair) for qq in qs]
        a = jnp.concatenate([lhs[h] for h in heads], axis=1).astype(_BF16)
        lo, hi = wo_rng[i]
        wait(wo_v.at[:, prio, pl.ds(lo, hi - lo)], S_WO + i)
        w = wo_v[:, prio, qs[0] * head_tiles:(qs[-1] + 1) * head_tiles]
        part = _dot(a, _untile(w, n_j))
        if i > 0:
            part = part + s_v[...]
        s_v[...] = part

    gb = jnp.broadcast_to(g, (sub, n_c))
    acc8 = [part[:, cb * _LANES:(cb + 1) * _LANES] for cb in range(n_j)]
    for i, (p, lo, t0, hi) in enumerate(wo_vpu):
        last = i == _N_WO_VPU - 1
        mult = []
        for t in range(t0 - q3, hi - q3):
            rb, cb = divmod(t, n_j)
            mt = col[p][rb * _SUB:(rb + 1) * _SUB]
            if last:
                mt = mt * gb[:, cb * _LANES:(cb + 1) * _LANES]
            mult.append(mt)
        if last:
            x8 = jnp.where(lax.broadcasted_iota(jnp.int32, (sub, n_c), 0) == 0,
                           jnp.broadcast_to(x, (sub, n_c)), 0.0)
            tot = jnp.concatenate(acc8, axis=1) * gb + x8
            acc8 = [tot[:, cb * _LANES:(cb + 1) * _LANES] for cb in range(n_j)]
        wait(wo_v.at[p, 1, pl.ds(lo, hi - lo)], S_WO + len(_WO_MXU) + i)
        w = wo_v[p, 1, t0:hi].astype(_F32)
        terms = [[a] for a in acc8]
        for k, t in enumerate(range(t0 - q3, hi - q3)):
            terms[t % n_j].append(w[k] * mult[k])
        acc8 = [_tree_sum(ts) for ts in terms]
    out = jnp.sum(jnp.concatenate(acc8, axis=1), axis=0, keepdims=True)
    o_ref[0] = out.astype(o_ref.dtype)


@jax.jit
def pallas_recurrent_scan__compressed_kv_cla__dense_activation_silu__decode_kernel(
    A_x: jax.Array,
    A_c_kv: jax.Array,
    A_w_q: jax.Array,
    A_w_uk: jax.Array,
    A_w_uv: jax.Array,
    A_w_o: jax.Array,
    B_x: jax.Array,
    B_w1: jax.Array,
    B_w2: jax.Array,
):
    del B_x
    b, s_q, m = A_x.shape
    _, s_k, d_c = A_c_kv.shape
    _, n_h, n_d = A_w_q.shape
    assert b == 1 and s_q == 1 and m == d_c and s_k % _KV_BLOCK == 0
    n_blk = s_k // _KV_BLOCK

    ckv = _tiles(A_c_kv.reshape(s_k, d_c)).reshape(_N_LANE, -1, _SUB, _LANES)
    wq, wuk, wuv = (w.reshape(-1, n_d) for w in (A_w_q, A_w_uk, A_w_uv))
    wo = _tiles(A_w_o.reshape(-1, m)).reshape(_N_LANE // 2, 2, -1, _SUB, _LANES)
    w1 = _tiles(B_w1.T)
    w2 = _tiles(B_w2)
    ops = (A_x, ckv, wq, wuk, wuv, wo, w1, w2)

    return pl.pallas_call(
        functools.partial(_kernel, eps=1e-5, n_h=n_h),
        in_specs=[pl.BlockSpec(memory_space=pl.ANY)] * len(ops),
        out_specs=pl.BlockSpec(memory_space=pltpu.VMEM),
        out_shape=jax.ShapeDtypeStruct(A_x.shape, A_x.dtype),
        scratch_shapes=[pltpu.VMEM(a.shape, a.dtype) for a in ops] + [
            pltpu.VMEM((_LANES, _LANES * n_h), _BF16),
            pltpu.VMEM((8, m), _F32),
            pltpu.SemaphoreType.DMA((10 + len(_WO_MXU) + _N_WO_VPU + n_blk,)),
        ],
        compiler_params=pltpu.CompilerParams(
            vmem_limit_bytes=96 * 1024 * 1024,
            disable_bounds_checks=True,
            disable_semaphore_checks=True),
    )(*ops)
```

```python
import functools

import jax
import jax.numpy as jnp
from jax import lax
import jax.experimental.pallas as pl
import jax.experimental.pallas.tpu as pltpu

_F32 = jnp.float32
_BF16 = jnp.bfloat16
_LANES = 128
_SUB = 8

_PIECE = 16
_SHIFT_A = 14
_SHIFT_B = 15
_N_LANE = 8
_KV_BLOCK = 1024
_LOOK_A = 2
_LOOK_B = 4


def _dot(a, b):
    return jnp.dot(a, b, preferred_element_type=_F32)


def _dot_nt(a, b):
    return lax.dot_general(a, b, (((1,), (1,)), ((), ())),
                           preferred_element_type=_F32)


def _silu(v):
    return v * jax.nn.sigmoid(v)


def _split(seq, n):
    q, r = divmod(len(seq), n)
    out, i = [], 0
    for k in range(n):
        m = q + (1 if k < r else 0)
        out.append(seq[i:i + m])
        i += m
    return out


def _round_robin(lanes):
    out = []
    for t in range(max(len(l) for l in lanes)):
        out.extend(l[t] for l in lanes if t < len(l))
    return out


def _tree_sum(xs):
    while len(xs) > 1:
        xs = [xs[i] + xs[i + 1] if i + 1 < len(xs) else xs[i]
              for i in range(0, len(xs), 2)]
    return xs[0]


def _cuts(lo, hi, shift):
    out = []
    while lo < hi:
        nxt = min(hi, lo + ((shift - lo - 1) % _PIECE) + 1)
        out.append((lo, nxt - lo))
        lo = nxt
    return out


def _tiles(a):
    r, c = a.shape
    a = a.reshape(r // _SUB, _SUB, c // _LANES, _LANES).transpose(0, 2, 1, 3)
    return a.reshape(-1, _SUB, _LANES)


def _untile(v, n_cb):
    v = v.reshape(-1, n_cb, _SUB, _LANES)
    return jnp.concatenate(
        [v[:, cb].reshape(-1, _LANES) for cb in range(n_cb)], axis=1)


_N_WO_MXU = 2
_N_WO_VPU = 9
_KV_ORDER = ((0, 4, 2, 6), (1, 5, 3, 7))


def _kernel(x_hbm, ckv_hbm, wq_hbm, wuk_hbm, wuv_hbm, wo_hbm, w1_hbm, w2_hbm,
            o_ref,
            x_v, ckv_v, wq_v, wuk_v, wuv_v, wo_v, w1_v, w2_v, e_v, s_v,
            sems, *, eps, n_h):
    n_c = x_v.shape[-1]
    n_d = wq_v.shape[-1]
    n_j = n_c // _LANES
    kj = _LANES * n_h
    lane_tiles = ckv_v.shape[1]
    blk_tiles = _KV_BLOCK // _N_LANE // _SUB * n_j
    n_blk = lane_tiles // blk_tiles
    rounds = blk_tiles // _PIECE
    half = rounds * _N_LANE // 2
    head_tiles = n_d // _SUB * n_j

    S_X, S_WQ, S_WUK, S_W1, S_W2, S_WUV, S_KV0, S_WO0 = 0, 1, 2, 6, 7, 8, 9, 10
    S_WO = 11
    S_KV = S_WO + _N_WO_MXU + _N_WO_VPU

    def row_pieces(src, dst, shift, sem_of):
        return [(src.at[pl.ds(t * _SUB, n * _SUB)],
                 dst.at[pl.ds(t * _SUB, n * _SUB)], sem_of(t))
                for t, n in _cuts(0, src.shape[0] // _SUB, shift)]

    def tile_pieces(src, dst, shift, s):
        return [(src.at[pl.ds(t, n)], dst.at[pl.ds(t, n)], s)
                for t, n in _cuts(0, src.shape[0], shift)]

    def kv_pieces(b, parity):
        out = []
        for r in range(rounds):
            t = b * blk_tiles + _SHIFT_A + r * _PIECE
            n = _PIECE
            if isinstance(b, int):
                n = min(n, lane_tiles - t)
            if n > 0:
                out += [(ckv_hbm.at[k, pl.ds(t, n)], ckv_v.at[k, pl.ds(t, n)],
                         S_KV + b) for k in _KV_ORDER[parity]]
        return out

    def start(piece, prio):
        src, dst, s = piece
        pltpu.make_async_copy(src, dst, sems.at[s]).start(priority=prio)

    def wait(buf, s):
        pltpu.make_async_copy(buf, buf, sems.at[s]).wait()

    def start_pairs(a, b):
        for t in range(max(len(a), len(b))):
            if t < len(a):
                start(a[t], 0)
            if t < len(b):
                start(b[t], 1)

    jt = kj // _SUB
    wq_p = row_pieces(wq_hbm, wq_v, _SHIFT_A, lambda t: S_WQ)
    wuk_p = row_pieces(wuk_hbm, wuk_v, _SHIFT_A, lambda t: S_WUK + t // jt)
    wuv_p = row_pieces(wuv_hbm, wuv_v, _SHIFT_A, lambda t: S_WUV)
    w1_p = tile_pieces(w1_hbm, w1_v, _SHIFT_B, S_W1)
    w2_p = tile_pieces(w2_hbm, w2_v, _SHIFT_B, S_W2)
    kv0_p = [(ckv_hbm.at[k, pl.ds(0, _SHIFT_A)], ckv_v.at[k, pl.ds(0, _SHIFT_A)],
              S_KV0) for k in range(_N_LANE)]
    wo_lane_tiles = wo_v.shape[2]
    n_pair = _N_LANE // 2

    def wo_pieces(p, par, lo, hi, s):
        return [(wo_hbm.at[p, par, pl.ds(t, n)], wo_v.at[p, par, pl.ds(t, n)],
                 s) for t, n in _cuts(lo, hi, _SHIFT_A)]

    wo0 = [wo_pieces(p, 0, 0, wo_lane_tiles, S_WO0) for p in range(n_pair)]
    g0 = _round_robin(_split(wq_p, 4) + _split(wuk_p, 4))
    l1 = _split(w1_p, 2)
    g1 = _round_robin(_split(wuv_p, 4) + [wo0[0] + wo0[1], wo0[2] + wo0[3]] + l1)
    n_ffn = 8 * len(l1[0])
    pre = g0 + g1 + kv0_p
    pre_a, pre_b = pre[1::2], pre[0::2]
    for b in range(_LOOK_A):
        pre_a = pre_a + kv_pieces(b, 0)
    for b in range(_LOOK_B):
        pre_b = pre_b + kv_pieces(b, 1)
    prime = len(pre_b) - len(pre_a)

    wo_a, wo_b, wo_rng = [], [], []
    for qq in range(_N_WO_MXU):
        lo = qq * head_tiles + (_SHIFT_A if qq else 0)
        hi = (qq + 1) * head_tiles + _SHIFT_A
        (wo_a if qq < 2 else wo_b).extend(_round_robin(
            [wo_pieces(p, 1, lo, hi, S_WO + qq) for p in range(n_pair)]))
        wo_rng.append((lo, hi))
    wo_vpu = []
    for qq in range(_N_WO_MXU, wo_lane_tiles // head_tiles):
        t0, t1 = qq * head_tiles, (qq + 1) * head_tiles
        for p in range(n_pair):
            wo_vpu.append((p, qq, t0 + _SHIFT_A,
                           min(t1 + _SHIFT_A, wo_lane_tiles), t0, t1))
    p, qq, lo, hi, t0, t1 = wo_vpu.pop()
    cut = lo + 2 * _PIECE
    wo_vpu += [(p, qq, lo, cut, t0, cut), (p, qq, cut, hi, cut, t1)]
    assert len(wo_vpu) == _N_WO_VPU
    for gi, (p, _, lo, hi, _, _) in enumerate(wo_vpu):
        wo_b.extend(wo_pieces(p, 1, lo, hi, S_WO + _N_WO_MXU + gi))

    n_main = n_blk - _LOOK_B - 1
    tail_a = sum([kv_pieces(b, 0) for b in range(n_main + _LOOK_A, n_blk)], [])
    tail_b = sum([kv_pieces(b, 1) for b in range(n_main + _LOOK_B, n_blk)], [])
    tail_a += wo_a
    tail_b += _round_robin(_split(w2_p, 2)) + wo_b

    issued = [0]

    def issue_to(n_a):
        n_a = min(n_a, len(pre_a))
        lo = issued[0]
        if n_a > lo:
            start_pairs(pre_a[lo:n_a], pre_b[prime + lo:prime + n_a])
            issued[0] = n_a

    pltpu.make_async_copy(x_hbm, x_v, sems.at[S_X]).start(priority=0)
    for p in pre_b[:prime]:
        start(p, 1)
    issue_to(22)

    e_row = lax.broadcasted_iota(jnp.int32, (_LANES, kj), 0)
    e_col = lax.broadcasted_iota(jnp.int32, (_LANES, kj), 1)
    e_v[...] = jnp.where(e_col // n_h == e_row, 1.0, 0.0).astype(_BF16)
    d_row = lax.broadcasted_iota(jnp.int32, (n_h, kj), 0)
    d_col = lax.broadcasted_iota(jnp.int32, (n_h, kj), 1)
    diag = (d_col % n_h) == d_row

    def w_block(w_ref, j):
        return w_ref[j * kj:(j + 1) * kj]

    n_a = _LANES // n_h
    hh = n_h // 2
    diag0 = diag[:, :_LANES]
    diag1 = diag[:, hh:hh + _LANES]

    def contract_major(c, w_ref):
        out = None
        for j in range(n_j):
            cj = pltpu.roll(c[:, j * _LANES:(j + 1) * _LANES], 0, 1,
                            stride=1, stride_axis=0).astype(_BF16)
            rs = [pltpu.roll(cj, (_LANES - r) % _LANES, 1) for r in range(hh)]
            zero = jnp.zeros_like(cj)
            x = jnp.concatenate(
                [jnp.where(d, r, zero) for r in rs for d in (diag0, diag1)],
                axis=1)
            w = w_block(w_ref, j).reshape(n_a, 2, hh, 2, hh, n_d)
            w = jnp.transpose(w, (2, 1, 0, 3, 4, 5))
            w = w.reshape(hh, 2, 2 * n_a, hh, n_d)
            w = jnp.concatenate(
                [w[:, 0], w[:, 1, 2 * n_a - 1:], w[:, 1, :2 * n_a - 1]], axis=1)
            part = _dot(x, w.reshape(kj, n_d))
            out = part if out is None else out + part
        return out

    issue_to(26)
    wait(x_v, S_X)
    x = x_v[0].astype(_F32)
    mu = jnp.mean(x, axis=-1, keepdims=True)
    xc = x - mu
    var = jnp.mean(xc * xc, axis=-1, keepdims=True)
    xn = (xc / jnp.sqrt(var + eps)).astype(_BF16)

    ahead = 30
    ptr = len(g0) // 2 + ahead
    issue_to(ptr)
    wait(wq_v, S_WQ)
    q = contract_major(jnp.broadcast_to(xn.astype(_F32), (n_h, n_c)),
                       wq_v).astype(_BF16)

    scale = n_d ** -0.5
    ts = []
    ptr += 10
    for j in range(n_j):
        issue_to(ptr)
        ptr += 6
        lo = j * jt + (_SHIFT_A if j else 0)
        hi = min((j + 1) * jt + _SHIFT_A, n_j * jt)
        wait(wuk_v.at[pl.ds(lo * _SUB, (hi - lo) * _SUB)], S_WUK + j)
        t = _dot_nt(q, w_block(wuk_v, j))
        ts.append(jnp.where(diag, t * scale, 0.0).astype(_BF16))
    issue_to(ptr)
    qa = _dot_nt(jnp.concatenate(ts, axis=0), e_v[...])
    q_abs = jnp.concatenate(
        [qa[j * n_h:(j + 1) * n_h] for j in range(n_j)], axis=1).astype(_BF16)

    ptr = max(ptr + 10, (len(g0) + n_ffn) // 2 + ahead)
    issue_to(ptr)
    wait(w1_v, S_W1)
    h1 = _silu(_dot_nt(xn, _untile(w1_v[...], n_j))).astype(_BF16)
    issue_to(len(pre_a))
    wait(ckv_v.at[:, pl.ds(0, _SHIFT_A)], S_KV0)

    def kv_step(i, carry):
        m, l, acc = carry

        @pl.when(i < n_main)
        def _():
            start_pairs(kv_pieces(i + _LOOK_A, 0), kv_pieces(i + _LOOK_B, 1))

        for c in range(n_main, n_blk):
            @pl.when(i == c)
            def _(c=c):
                k0 = (c - n_main) * half
                start_pairs(tail_a[k0:k0 + half], tail_b[k0:k0 + half])

        t0 = i * blk_tiles

        @pl.when(i < n_blk - 1)
        def _():
            wait(ckv_v.at[:, pl.ds(t0 + _SHIFT_A, blk_tiles)], S_KV + i)

        @pl.when(i == n_blk - 1)
        def _():
            wait(ckv_v.at[:, pl.ds(lane_tiles - blk_tiles + _SHIFT_A,
                                   blk_tiles - _SHIFT_A)], S_KV + n_blk - 1)

        kv = _untile(ckv_v[:, pl.ds(t0, blk_tiles)], n_j)
        s = _dot_nt(q_abs, kv)
        m_new = jnp.maximum(m, jnp.max(s, axis=1, keepdims=True))
        alpha = jnp.exp(m - m_new)
        p = jnp.exp(s - m_new)
        l = alpha * l + jnp.sum(p, axis=1, keepdims=True)
        acc = alpha * acc + _dot(p.astype(_BF16), kv)
        return m_new, l, acc

    m0 = jnp.full((n_h, 1), -jnp.inf, _F32)
    l0 = jnp.zeros((n_h, 1), _F32)
    a0 = jnp.zeros((n_h, n_c), _F32)
    _, l, acc = lax.fori_loop(0, n_blk, kv_step, (m0, l0, a0))
    k0 = (n_blk - n_main) * half
    start_pairs(tail_a[k0:], tail_b[k0:])
    ctx_c = acc / l

    wait(wuv_v, S_WUV)
    wait(wo_v.at[:, 0], S_WO0)
    ctx = contract_major(ctx_c, wuv_v)

    sub = 8
    row = lax.broadcasted_iota(jnp.int32, (sub, n_d), 0)
    lhs = [jnp.where(row == h % sub,
                     ctx[(h // sub) * sub:(h // sub + 1) * sub], 0.0)
           for h in range(n_h)]
    per = n_h // _N_LANE
    ctx_r = ctx.astype(_BF16).astype(_F32)
    col = {}
    for p, qq, _, _, _, _ in wo_vpu:
        h = (2 * p + 1) * per + qq
        col[p, qq] = jnp.transpose(
            jnp.broadcast_to(ctx_r[h:h + 1], (n_d, n_d)))
    a = jnp.concatenate([lhs[2 * p * per + qq] for p in range(n_pair)
                         for qq in range(per)], axis=1).astype(_BF16)
    s_v[...] = _dot(a, _untile(wo_v[:, 0], n_j))
    for qq in range(_N_WO_MXU):
        a = jnp.concatenate([lhs[(2 * p + 1) * per + qq]
                             for p in range(n_pair)], axis=1).astype(_BF16)
        lo, hi = wo_rng[qq]
        wait(wo_v.at[:, 1, pl.ds(lo, hi - lo)], S_WO + qq)
        w = wo_v[:, 1, qq * head_tiles:(qq + 1) * head_tiles]
        part = _dot(a, _untile(w, n_j)) + s_v[...]
        s_v[...] = part

    wait(w2_v, S_W2)
    g = _silu(_dot(h1, _untile(w2_v[...], n_j)))
    gb = jnp.broadcast_to(g, (sub, n_c))
    acc8 = [part[:, cb * _LANES:(cb + 1) * _LANES] for cb in range(n_j)]
    for i, (p, qq, lo, hi, t0, t1) in enumerate(wo_vpu):
        last = i == _N_WO_VPU - 1
        mult = []
        for t in range(t0, t1):
            rb, cb = divmod(t % head_tiles, n_j)
            mt = col[p, qq][rb * _SUB:(rb + 1) * _SUB]
            if last:
                mt = mt * gb[:, cb * _LANES:(cb + 1) * _LANES]
            mult.append(mt)
        if last:
            x8 = jnp.where(lax.broadcasted_iota(jnp.int32, (sub, n_c), 0) == 0,
                           jnp.broadcast_to(x, (sub, n_c)), 0.0)
            tot = jnp.concatenate(acc8, axis=1) * gb + x8
            acc8 = [tot[:, cb * _LANES:(cb + 1) * _LANES] for cb in range(n_j)]
        wait(wo_v.at[p, 1, pl.ds(lo, hi - lo)], S_WO + _N_WO_MXU + i)
        w = wo_v[p, 1, t0:t1].astype(_F32)
        terms = [[a] for a in acc8]
        for k, t in enumerate(range(t0, t1)):
            terms[t % n_j].append(w[k] * mult[k])
        acc8 = [_tree_sum(ts) for ts in terms]
    out = jnp.sum(jnp.concatenate(acc8, axis=1), axis=0, keepdims=True)
    o_ref[0] = out.astype(o_ref.dtype)


@jax.jit
def pallas_recurrent_scan__compressed_kv_cla__dense_activation_silu__decode_kernel(
    A_x: jax.Array,
    A_c_kv: jax.Array,
    A_w_q: jax.Array,
    A_w_uk: jax.Array,
    A_w_uv: jax.Array,
    A_w_o: jax.Array,
    B_x: jax.Array,
    B_w1: jax.Array,
    B_w2: jax.Array,
):
    del B_x
    b, s_q, m = A_x.shape
    _, s_k, d_c = A_c_kv.shape
    _, n_h, n_d = A_w_q.shape
    assert b == 1 and s_q == 1 and m == d_c and s_k % _KV_BLOCK == 0
    n_blk = s_k // _KV_BLOCK

    ckv = _tiles(A_c_kv.reshape(s_k, d_c)).reshape(_N_LANE, -1, _SUB, _LANES)
    wq, wuk, wuv = (w.reshape(-1, n_d) for w in (A_w_q, A_w_uk, A_w_uv))
    wo = _tiles(A_w_o.reshape(-1, m)).reshape(_N_LANE // 2, 2, -1, _SUB, _LANES)
    w1 = _tiles(B_w1.T)
    w2 = _tiles(B_w2)
    ops = (A_x, ckv, wq, wuk, wuv, wo, w1, w2)

    return pl.pallas_call(
        functools.partial(_kernel, eps=1e-5, n_h=n_h),
        in_specs=[pl.BlockSpec(memory_space=pl.ANY)] * len(ops),
        out_specs=pl.BlockSpec(memory_space=pltpu.VMEM),
        out_shape=jax.ShapeDtypeStruct(A_x.shape, A_x.dtype),
        scratch_shapes=[pltpu.VMEM(a.shape, a.dtype) for a in ops] + [
            pltpu.VMEM((_LANES, _LANES * n_h), _BF16),
            pltpu.VMEM((8, m), _F32),
            pltpu.SemaphoreType.DMA((11 + _N_WO_MXU + _N_WO_VPU + n_blk,)),
        ],
        compiler_params=pltpu.CompilerParams(
            vmem_limit_bytes=96 * 1024 * 1024,
            disable_bounds_checks=True,
            disable_semaphore_checks=True),
    )(*ops)
```

```python
import functools

import jax
import jax.numpy as jnp
from jax import lax
import jax.experimental.pallas as pl
import jax.experimental.pallas.tpu as pltpu

_F32 = jnp.float32
_BF16 = jnp.bfloat16
_LANES = 128
_SUB = 8

_PIECE = 16
_SHIFT_A = 14
_SHIFT_B = 15
_N_LANE = 8
_KV_BLOCK = 1024
_LOOK_A = 2
_LOOK_B = 4


def _dot(a, b):
    return jnp.dot(a, b, preferred_element_type=_F32)


def _dot_nt(a, b):
    return lax.dot_general(a, b, (((1,), (1,)), ((), ())),
                           preferred_element_type=_F32)


def _silu(v):
    return v * jax.nn.sigmoid(v)


def _split(seq, n):
    q, r = divmod(len(seq), n)
    out, i = [], 0
    for k in range(n):
        m = q + (1 if k < r else 0)
        out.append(seq[i:i + m])
        i += m
    return out


def _round_robin(lanes):
    out = []
    for t in range(max(len(l) for l in lanes)):
        out.extend(l[t] for l in lanes if t < len(l))
    return out


def _tree_sum(xs):
    while len(xs) > 1:
        xs = [xs[i] + xs[i + 1] if i + 1 < len(xs) else xs[i]
              for i in range(0, len(xs), 2)]
    return xs[0]


def _cuts(lo, hi, shift):
    out = []
    while lo < hi:
        nxt = min(hi, lo + ((shift - lo - 1) % _PIECE) + 1)
        out.append((lo, nxt - lo))
        lo = nxt
    return out


def _tiles(a):
    r, c = a.shape
    a = a.reshape(r // _SUB, _SUB, c // _LANES, _LANES).transpose(0, 2, 1, 3)
    return a.reshape(-1, _SUB, _LANES)


def _untile(v, n_cb):
    v = v.reshape(-1, n_cb, _SUB, _LANES)
    return jnp.concatenate(
        [v[:, cb].reshape(-1, _LANES) for cb in range(n_cb)], axis=1)


_N_WO_MXU = 2
_N_WO_VPU = 9
_KV_ORDER = ((0, 4, 2, 6), (1, 5, 3, 7))


def _kernel(x_hbm, ckv_hbm, wq_hbm, wuk_hbm, wuv_hbm, wo_hbm, w1_hbm, w2_hbm,
            o_ref,
            x_v, ckv_v, wq_v, wuk_v, wuv_v, wo_v, w1_v, w2_v, e_v, s_v,
            sems, *, eps, n_h):
    n_c = x_v.shape[-1]
    n_d = wq_v.shape[-1]
    n_j = n_c // _LANES
    kj = _LANES * n_h
    lane_tiles = ckv_v.shape[1]
    blk_tiles = _KV_BLOCK // _N_LANE // _SUB * n_j
    n_blk = lane_tiles // blk_tiles
    rounds = blk_tiles // _PIECE
    half = rounds * _N_LANE // 2
    head_tiles = n_d // _SUB * n_j

    S_X, S_WQ, S_WUK, S_W1, S_W2, S_WUV, S_KV0, S_WO0 = 0, 1, 2, 6, 7, 8, 9, 10
    S_WO = 11
    S_KV = S_WO + _N_WO_MXU + _N_WO_VPU

    def row_pieces(src, dst, shift, sem_of):
        return [(src.at[pl.ds(t * _SUB, n * _SUB)],
                 dst.at[pl.ds(t * _SUB, n * _SUB)], sem_of(t))
                for t, n in _cuts(0, src.shape[0] // _SUB, shift)]

    def tile_pieces(src, dst, shift, s):
        return [(src.at[pl.ds(t, n)], dst.at[pl.ds(t, n)], s)
                for t, n in _cuts(0, src.shape[0], shift)]

    def kv_pieces(b, parity):
        out = []
        for r in range(rounds):
            t = b * blk_tiles + _SHIFT_A + r * _PIECE
            n = _PIECE
            if isinstance(b, int):
                n = min(n, lane_tiles - t)
            if n > 0:
                out += [(ckv_hbm.at[k, pl.ds(t, n)], ckv_v.at[k, pl.ds(t, n)],
                         S_KV + b) for k in _KV_ORDER[parity]]
        return out

    def start(piece, prio):
        src, dst, s = piece
        pltpu.make_async_copy(src, dst, sems.at[s]).start(priority=prio)

    def wait(buf, s):
        pltpu.make_async_copy(buf, buf, sems.at[s]).wait()

    def start_pairs(a, b):
        for t in range(max(len(a), len(b))):
            if t < len(a):
                start(a[t], 0)
            if t < len(b):
                start(b[t], 1)

    jt = kj // _SUB
    wq_p = row_pieces(wq_hbm, wq_v, _SHIFT_A, lambda t: S_WQ)
    wuk_p = row_pieces(wuk_hbm, wuk_v, _SHIFT_A, lambda t: S_WUK + t // jt)
    wuv_p = row_pieces(wuv_hbm, wuv_v, _SHIFT_A, lambda t: S_WUV)
    w1_p = tile_pieces(w1_hbm, w1_v, _SHIFT_B, S_W1)
    w2_p = tile_pieces(w2_hbm, w2_v, _SHIFT_B, S_W2)
    kv0_p = [(ckv_hbm.at[k, pl.ds(0, _SHIFT_A)], ckv_v.at[k, pl.ds(0, _SHIFT_A)],
              S_KV0) for k in range(_N_LANE)]
    wo_lane_tiles = wo_v.shape[2]
    n_pair = _N_LANE // 2

    def wo_pieces(p, par, lo, hi, s):
        return [(wo_hbm.at[p, par, pl.ds(t, n)], wo_v.at[p, par, pl.ds(t, n)],
                 s) for t, n in _cuts(lo, hi, _SHIFT_A)]

    wo0 = [wo_pieces(p, 0, 0, wo_lane_tiles, S_WO0) for p in range(n_pair)]
    g0 = _round_robin(_split(wq_p, 4) + _split(wuk_p, 4))
    l1 = _split(w1_p, 2)
    g1 = _round_robin(_split(wuv_p, 4) + [wo0[0] + wo0[1], wo0[2] + wo0[3]] + l1)
    n_ffn = 8 * len(l1[0])
    pre = g0 + g1 + kv0_p
    pre_a, pre_b = pre[1::2], pre[0::2]
    for b in range(_LOOK_A):
        pre_a = pre_a + kv_pieces(b, 0)
    for b in range(_LOOK_B):
        pre_b = pre_b + kv_pieces(b, 1)
    prime = len(pre_b) - len(pre_a)

    wo_a, wo_b, wo_rng = [], [], []
    for qq in range(_N_WO_MXU):
        lo = qq * head_tiles + (_SHIFT_A if qq else 0)
        hi = (qq + 1) * head_tiles + _SHIFT_A
        wo_a.extend(_round_robin(
            [wo_pieces(p, 1, lo, hi, S_WO + qq) for p in range(n_pair)]))
        wo_rng.append((lo, hi))
    wo_vpu = []
    for qq in range(_N_WO_MXU, wo_lane_tiles // head_tiles):
        t0, t1 = qq * head_tiles, (qq + 1) * head_tiles
        for p in range(n_pair):
            wo_vpu.append((p, qq, t0 + _SHIFT_A,
                           min(t1 + _SHIFT_A, wo_lane_tiles), t0, t1))
    p, qq, lo, hi, t0, t1 = wo_vpu.pop()
    cut = lo + 2 * _PIECE
    wo_vpu += [(p, qq, lo, cut, t0, cut), (p, qq, cut, hi, cut, t1)]
    assert len(wo_vpu) == _N_WO_VPU
    for gi, (p, _, lo, hi, _, _) in enumerate(wo_vpu):
        wo_b.extend(wo_pieces(p, 1, lo, hi, S_WO + _N_WO_MXU + gi))

    n_main = n_blk - _LOOK_B - 1
    tail_a = sum([kv_pieces(b, 0) for b in range(n_main + _LOOK_A, n_blk)], [])
    tail_b = sum([kv_pieces(b, 1) for b in range(n_main + _LOOK_B, n_blk)], [])
    tail_a += wo_a
    tail_b += _round_robin(_split(w2_p, 2)) + wo_b

    issued = [0]

    def issue_to(n_a):
        n_a = min(n_a, len(pre_a))
        lo = issued[0]
        if n_a > lo:
            start_pairs(pre_a[lo:n_a], pre_b[prime + lo:prime + n_a])
            issued[0] = n_a

    for p in pre_b[:8]:
        start(p, 1)
    start((x_hbm, x_v, S_X), 0)
    for p in pre_b[8:prime]:
        start(p, 1)
    issue_to(22)

    e_row = lax.broadcasted_iota(jnp.int32, (_LANES, kj), 0)
    e_col = lax.broadcasted_iota(jnp.int32, (_LANES, kj), 1)
    e_v[...] = jnp.where(e_col // n_h == e_row, 1.0, 0.0).astype(_BF16)
    d_row = lax.broadcasted_iota(jnp.int32, (n_h, kj), 0)
    d_col = lax.broadcasted_iota(jnp.int32, (n_h, kj), 1)
    diag = (d_col % n_h) == d_row

    def w_block(w_ref, j):
        return w_ref[j * kj:(j + 1) * kj]

    n_a = _LANES // n_h
    hh = n_h // 2
    diag0 = diag[:, :_LANES]
    diag1 = diag[:, hh:hh + _LANES]

    def contract_major(c, w_ref):
        out = None
        for j in range(n_j):
            cj = pltpu.roll(c[:, j * _LANES:(j + 1) * _LANES], 0, 1,
                            stride=1, stride_axis=0).astype(_BF16)
            rs = [pltpu.roll(cj, (_LANES - r) % _LANES, 1) for r in range(hh)]
            zero = jnp.zeros_like(cj)
            x = jnp.concatenate(
                [jnp.where(d, r, zero) for r in rs for d in (diag0, diag1)],
                axis=1)
            w = w_block(w_ref, j).reshape(n_a, 2, hh, 2, hh, n_d)
            w = jnp.transpose(w, (2, 1, 0, 3, 4, 5))
            w = w.reshape(hh, 2, 2 * n_a, hh, n_d)
            w = jnp.concatenate(
                [w[:, 0], w[:, 1, 2 * n_a - 1:], w[:, 1, :2 * n_a - 1]], axis=1)
            part = _dot(x, w.reshape(kj, n_d))
            out = part if out is None else out + part
        return out

    issue_to(26)
    wait(x_v, S_X)
    x = x_v[0].astype(_F32)
    mu = jnp.mean(x, axis=-1, keepdims=True)
    xc = x - mu
    var = jnp.mean(xc * xc, axis=-1, keepdims=True)
    xn = (xc / jnp.sqrt(var + eps)).astype(_BF16)

    ahead = 30
    ptr = len(g0) // 2 + ahead
    issue_to(ptr)
    wait(wq_v, S_WQ)
    q = contract_major(jnp.broadcast_to(xn.astype(_F32), (n_h, n_c)),
                       wq_v).astype(_BF16)

    scale = n_d ** -0.5
    ts = []
    ptr += 14
    for j in range(n_j):
        issue_to(ptr)
        ptr += 6
        lo = j * jt + (_SHIFT_A if j else 0)
        hi = min((j + 1) * jt + _SHIFT_A, n_j * jt)
        wait(wuk_v.at[pl.ds(lo * _SUB, (hi - lo) * _SUB)], S_WUK + j)
        t = _dot_nt(q, w_block(wuk_v, j))
        ts.append(jnp.where(diag, t * scale, 0.0).astype(_BF16))
    issue_to(ptr)
    qa = _dot_nt(jnp.concatenate(ts, axis=0), e_v[...])
    q_abs = jnp.concatenate(
        [qa[j * n_h:(j + 1) * n_h] for j in range(n_j)], axis=1).astype(_BF16)

    ptr = max(ptr + 10, (len(g0) + n_ffn) // 2 + ahead)
    issue_to(ptr)
    wait(w1_v, S_W1)
    h1 = _silu(_dot_nt(xn, _untile(w1_v[...], n_j))).astype(_BF16)
    issue_to(len(pre_a))
    wait(ckv_v.at[:, pl.ds(0, _SHIFT_A)], S_KV0)

    def kv_step(i, carry):
        m, l, acc = carry

        @pl.when(i < n_main)
        def _():
            start_pairs(kv_pieces(i + _LOOK_A, 0), kv_pieces(i + _LOOK_B, 1))

        for c in range(n_main, n_blk):
            @pl.when(i == c)
            def _(c=c):
                k0 = (c - n_main) * half
                start_pairs(tail_a[k0:k0 + half], tail_b[k0:k0 + half])

        t0 = i * blk_tiles

        @pl.when(i < n_blk - 1)
        def _():
            wait(ckv_v.at[:, pl.ds(t0 + _SHIFT_A, blk_tiles)], S_KV + i)

        @pl.when(i == n_blk - 1)
        def _():
            wait(ckv_v.at[:, pl.ds(lane_tiles - blk_tiles + _SHIFT_A,
                                   blk_tiles - _SHIFT_A)], S_KV + n_blk - 1)

        kv = _untile(ckv_v[:, pl.ds(t0, blk_tiles)], n_j)
        s = _dot_nt(q_abs, kv)
        m_new = jnp.maximum(m, jnp.max(s, axis=1, keepdims=True))
        alpha = jnp.exp(m - m_new)
        p = jnp.exp(s - m_new)
        l = alpha * l + jnp.sum(p, axis=1, keepdims=True)
        acc = alpha * acc + _dot(p.astype(_BF16), kv)
        return m_new, l, acc

    m0 = jnp.full((n_h, 1), -jnp.inf, _F32)
    l0 = jnp.zeros((n_h, 1), _F32)
    a0 = jnp.zeros((n_h, n_c), _F32)
    _, l, acc = lax.fori_loop(0, n_blk, kv_step, (m0, l0, a0))
    k0 = (n_blk - n_main) * half
    start_pairs(tail_a[k0:], tail_b[k0:])
    ctx_c = acc / l

    wait(wuv_v, S_WUV)
    wait(wo_v.at[:, 0], S_WO0)
    ctx = contract_major(ctx_c, wuv_v)

    sub = 8
    row = lax.broadcasted_iota(jnp.int32, (sub, n_d), 0)
    lhs = [jnp.where(row == h % sub,
                     ctx[(h // sub) * sub:(h // sub + 1) * sub], 0.0)
           for h in range(n_h)]
    per = n_h // _N_LANE
    ctx_r = ctx.astype(_BF16).astype(_F32)
    col = {}
    for p, qq, _, _, _, _ in wo_vpu:
        h = (2 * p + 1) * per + qq
        col[p, qq] = jnp.transpose(
            jnp.broadcast_to(ctx_r[h:h + 1], (n_d, n_d)))
    a = jnp.concatenate([lhs[2 * p * per + qq] for p in range(n_pair)
                         for qq in range(per)], axis=1).astype(_BF16)
    s_v[...] = _dot(a, _untile(wo_v[:, 0], n_j))
    for qq in range(_N_WO_MXU):
        a = jnp.concatenate([lhs[(2 * p + 1) * per + qq]
                             for p in range(n_pair)], axis=1).astype(_BF16)
        lo, hi = wo_rng[qq]
        wait(wo_v.at[:, 1, pl.ds(lo, hi - lo)], S_WO + qq)
        w = wo_v[:, 1, qq * head_tiles:(qq + 1) * head_tiles]
        part = _dot(a, _untile(w, n_j)) + s_v[...]
        s_v[...] = part

    wait(w2_v, S_W2)
    g = _silu(_dot(h1, _untile(w2_v[...], n_j)))
    gb = jnp.broadcast_to(g, (sub, n_c))
    acc8 = [part[:, cb * _LANES:(cb + 1) * _LANES] for cb in range(n_j)]
    for i, (p, qq, lo, hi, t0, t1) in enumerate(wo_vpu):
        last = i == _N_WO_VPU - 1
        mult = []
        for t in range(t0, t1):
            rb, cb = divmod(t % head_tiles, n_j)
            mt = col[p, qq][rb * _SUB:(rb + 1) * _SUB]
            if last:
                mt = mt * gb[:, cb * _LANES:(cb + 1) * _LANES]
            mult.append(mt)
        if last:
            x8 = jnp.where(lax.broadcasted_iota(jnp.int32, (sub, n_c), 0) == 0,
                           jnp.broadcast_to(x, (sub, n_c)), 0.0)
            tot = jnp.concatenate(acc8, axis=1) * gb + x8
            acc8 = [tot[:, cb * _LANES:(cb + 1) * _LANES] for cb in range(n_j)]
        wait(wo_v.at[p, 1, pl.ds(lo, hi - lo)], S_WO + _N_WO_MXU + i)
        w = wo_v[p, 1, t0:t1].astype(_F32)
        terms = [[a] for a in acc8]
        for k, t in enumerate(range(t0, t1)):
            terms[t % n_j].append(w[k] * mult[k])
        acc8 = [_tree_sum(ts) for ts in terms]
    out = jnp.sum(jnp.concatenate(acc8, axis=1), axis=0, keepdims=True)
    o_ref[0] = out.astype(o_ref.dtype)


@jax.jit
def pallas_recurrent_scan__compressed_kv_cla__dense_activation_silu__decode_kernel(
    A_x: jax.Array,
    A_c_kv: jax.Array,
    A_w_q: jax.Array,
    A_w_uk: jax.Array,
    A_w_uv: jax.Array,
    A_w_o: jax.Array,
    B_x: jax.Array,
    B_w1: jax.Array,
    B_w2: jax.Array,
):
    del B_x
    b, s_q, m = A_x.shape
    _, s_k, d_c = A_c_kv.shape
    _, n_h, n_d = A_w_q.shape
    assert b == 1 and s_q == 1 and m == d_c and s_k % _KV_BLOCK == 0
    n_blk = s_k // _KV_BLOCK

    ckv = _tiles(A_c_kv.reshape(s_k, d_c)).reshape(_N_LANE, -1, _SUB, _LANES)
    wq, wuk, wuv = (w.reshape(-1, n_d) for w in (A_w_q, A_w_uk, A_w_uv))
    wo = _tiles(A_w_o.reshape(-1, m)).reshape(_N_LANE // 2, 2, -1, _SUB, _LANES)
    w1 = _tiles(B_w1.T)
    w2 = _tiles(B_w2)
    ops = (A_x, ckv, wq, wuk, wuv, wo, w1, w2)

    return pl.pallas_call(
        functools.partial(_kernel, eps=1e-5, n_h=n_h),
        in_specs=[pl.BlockSpec(memory_space=pl.ANY)] * len(ops),
        out_specs=pl.BlockSpec(memory_space=pltpu.VMEM),
        out_shape=jax.ShapeDtypeStruct(A_x.shape, A_x.dtype),
        scratch_shapes=[pltpu.VMEM(a.shape, a.dtype) for a in ops] + [
            pltpu.VMEM((_LANES, _LANES * n_h), _BF16),
            pltpu.VMEM((8, m), _F32),
            pltpu.SemaphoreType.DMA((11 + _N_WO_MXU + _N_WO_VPU + n_blk,)),
        ],
        compiler_params=pltpu.CompilerParams(
            vmem_limit_bytes=96 * 1024 * 1024,
            disable_bounds_checks=True,
            disable_semaphore_checks=True),
    )(*ops)
```

```python
import functools

import jax
import jax.numpy as jnp
from jax import lax
import jax.experimental.pallas as pl
import jax.experimental.pallas.tpu as pltpu

_F32 = jnp.float32
_BF16 = jnp.bfloat16
_LANES = 128
_SUB = 8

_PIECE = 16
_SHIFT_A = 14
_SHIFT_B = 15
_N_LANE = 8
_KV_BLOCK = 1024
_LOOK_A = 2
_LOOK_B = 4


def _dot(a, b):
    return jnp.dot(a, b, preferred_element_type=_F32)


def _dot_nt(a, b):
    return lax.dot_general(a, b, (((1,), (1,)), ((), ())),
                           preferred_element_type=_F32)


def _silu(v):
    return v * jax.nn.sigmoid(v)


def _split(seq, n):
    q, r = divmod(len(seq), n)
    out, i = [], 0
    for k in range(n):
        m = q + (1 if k < r else 0)
        out.append(seq[i:i + m])
        i += m
    return out


def _round_robin(lanes):
    out = []
    for t in range(max(len(l) for l in lanes)):
        out.extend(l[t] for l in lanes if t < len(l))
    return out


def _tree_sum(xs):
    while len(xs) > 1:
        xs = [xs[i] + xs[i + 1] if i + 1 < len(xs) else xs[i]
              for i in range(0, len(xs), 2)]
    return xs[0]


def _cuts(lo, hi, shift):
    out = []
    while lo < hi:
        nxt = min(hi, lo + ((shift - lo - 1) % _PIECE) + 1)
        out.append((lo, nxt - lo))
        lo = nxt
    return out


def _tiles(a):
    r, c = a.shape
    a = a.reshape(r // _SUB, _SUB, c // _LANES, _LANES).transpose(0, 2, 1, 3)
    return a.reshape(-1, _SUB, _LANES)


def _untile(v, n_cb):
    v = v.reshape(-1, n_cb, _SUB, _LANES)
    return jnp.concatenate(
        [v[:, cb].reshape(-1, _LANES) for cb in range(n_cb)], axis=1)


_N_WO_MXU = 2
_N_WO_VPU = 9
_KV_ORDER = ((0, 4, 2, 6), (1, 5, 3, 7))


def _kernel(x_hbm, ckv_hbm, wq_hbm, wuk_hbm, wuv_hbm, wo_hbm, w1_hbm, w2_hbm,
            o_ref,
            x_v, ckv_v, wq_v, wuk_v, wuv_v, wo_v, w1_v, w2_v, e_v, s_v,
            sems, *, eps, n_h):
    n_c = x_v.shape[-1]
    n_d = wq_v.shape[-1]
    n_j = n_c // _LANES
    kj = _LANES * n_h
    lane_tiles = ckv_v.shape[1]
    blk_tiles = _KV_BLOCK // _N_LANE // _SUB * n_j
    n_blk = lane_tiles // blk_tiles
    rounds = blk_tiles // _PIECE
    half = rounds * _N_LANE // 2
    head_tiles = n_d // _SUB * n_j

    S_X, S_WQ, S_WUK, S_W1, S_W2, S_WUV, S_KV0, S_WO0 = 0, 1, 2, 6, 7, 8, 9, 10
    S_WO = 11
    S_KV = S_WO + _N_WO_MXU + _N_WO_VPU

    def row_pieces(src, dst, shift, sem_of):
        return [(src.at[pl.ds(t * _SUB, n * _SUB)],
                 dst.at[pl.ds(t * _SUB, n * _SUB)], sem_of(t))
                for t, n in _cuts(0, src.shape[0] // _SUB, shift)]

    def tile_pieces(src, dst, shift, s):
        return [(src.at[pl.ds(t, n)], dst.at[pl.ds(t, n)], s)
                for t, n in _cuts(0, src.shape[0], shift)]

    def kv_pieces(b, parity):
        out = []
        for r in range(rounds):
            t = b * blk_tiles + _SHIFT_A + r * _PIECE
            n = _PIECE
            if isinstance(b, int):
                n = min(n, lane_tiles - t)
            if n > 0:
                out += [(ckv_hbm.at[k, pl.ds(t, n)], ckv_v.at[k, pl.ds(t, n)],
                         S_KV + b) for k in _KV_ORDER[parity]]
        return out

    def start(piece, prio):
        src, dst, s = piece
        pltpu.make_async_copy(src, dst, sems.at[s]).start(priority=prio)

    def wait(buf, s):
        pltpu.make_async_copy(buf, buf, sems.at[s]).wait()

    def start_pairs(a, b):
        for t in range(max(len(a), len(b))):
            if t < len(a):
                start(a[t], 0)
            if t < len(b):
                start(b[t], 1)

    jt = kj // _SUB
    wq_p = row_pieces(wq_hbm, wq_v, _SHIFT_A, lambda t: S_WQ)
    wuk_p = row_pieces(wuk_hbm, wuk_v, _SHIFT_A, lambda t: S_WUK + t // jt)
    wuv_p = row_pieces(wuv_hbm, wuv_v, _SHIFT_A, lambda t: S_WUV)
    w1_p = tile_pieces(w1_hbm, w1_v, _SHIFT_B, S_W1)
    w2_p = tile_pieces(w2_hbm, w2_v, _SHIFT_B, S_W2)
    kv0_p = [(ckv_hbm.at[k, pl.ds(0, _SHIFT_A)], ckv_v.at[k, pl.ds(0, _SHIFT_A)],
              S_KV0) for k in range(_N_LANE)]
    wo_lane_tiles = wo_v.shape[2]
    n_pair = _N_LANE // 2

    def wo_pieces(p, par, lo, hi, s):
        return [(wo_hbm.at[p, par, pl.ds(t, n)], wo_v.at[p, par, pl.ds(t, n)],
                 s) for t, n in _cuts(lo, hi, _SHIFT_A)]

    wo0 = [wo_pieces(p, 0, 0, wo_lane_tiles, S_WO0) for p in range(n_pair)]
    g0 = _round_robin(_split(wq_p, 4) + _split(wuk_p, 4))
    l1 = _split(w1_p, 2)
    g1 = _round_robin(_split(wuv_p, 4) + [wo0[0] + wo0[1], wo0[2] + wo0[3]] + l1)
    n_ffn = 8 * len(l1[0])
    pre = g0 + g1 + kv0_p
    pre_a, pre_b = pre[1::2], pre[0::2]
    for b in range(_LOOK_A):
        pre_a = pre_a + kv_pieces(b, 0)
    for b in range(_LOOK_B):
        pre_b = pre_b + kv_pieces(b, 1)
    prime = len(pre_b) - len(pre_a)

    wo_a, wo_b, wo_rng = [], [], []
    for qq in range(_N_WO_MXU):
        lo = qq * head_tiles + (_SHIFT_A if qq else 0)
        hi = (qq + 1) * head_tiles + _SHIFT_A
        wo_a.extend(_round_robin(
            [wo_pieces(p, 1, lo, hi, S_WO + qq) for p in range(n_pair)]))
        wo_rng.append((lo, hi))
    wo_vpu = []
    for qq in range(_N_WO_MXU, wo_lane_tiles // head_tiles):
        t0, t1 = qq * head_tiles, (qq + 1) * head_tiles
        for p in range(n_pair):
            wo_vpu.append((p, qq, t0 + _SHIFT_A,
                           min(t1 + _SHIFT_A, wo_lane_tiles), t0, t1))
    p, qq, lo, hi, t0, t1 = wo_vpu.pop()
    cut = lo + 2 * _PIECE
    wo_vpu += [(p, qq, lo, cut, t0, cut), (p, qq, cut, hi, cut, t1)]
    assert len(wo_vpu) == _N_WO_VPU
    for gi, (p, _, lo, hi, _, _) in enumerate(wo_vpu):
        wo_b.extend(wo_pieces(p, 1, lo, hi, S_WO + _N_WO_MXU + gi))

    n_main = n_blk - _LOOK_B - 1
    tail_a = sum([kv_pieces(b, 0) for b in range(n_main + _LOOK_A, n_blk)], [])
    tail_b = sum([kv_pieces(b, 1) for b in range(n_main + _LOOK_B, n_blk)], [])
    tail_a += wo_a
    tail_b += _round_robin(_split(w2_p, 2)) + wo_b

    issued = [0]

    def issue_to(n_a):
        n_a = min(n_a, len(pre_a))
        lo = issued[0]
        if n_a > lo:
            start_pairs(pre_a[lo:n_a], pre_b[prime + lo:prime + n_a])
            issued[0] = n_a

    for p in pre_b[:8]:
        start(p, 1)
    start((x_hbm, x_v, S_X), 0)
    for p in pre_b[8:prime]:
        start(p, 1)
    issue_to(22)

    e_row = lax.broadcasted_iota(jnp.int32, (_LANES, kj), 0)
    e_col = lax.broadcasted_iota(jnp.int32, (_LANES, kj), 1)
    e_v[...] = jnp.where(e_col // n_h == e_row, 1.0, 0.0).astype(_BF16)
    d_row = lax.broadcasted_iota(jnp.int32, (n_h, kj), 0)
    d_col = lax.broadcasted_iota(jnp.int32, (n_h, kj), 1)
    diag = (d_col % n_h) == d_row

    def w_block(w_ref, j):
        return w_ref[j * kj:(j + 1) * kj]

    n_a = _LANES // n_h
    hh = n_h // 2
    diag0 = diag[:, :_LANES]
    diag1 = diag[:, hh:hh + _LANES]

    def contract_major(c, w_ref):
        out = None
        for j in range(n_j):
            cj = pltpu.roll(c[:, j * _LANES:(j + 1) * _LANES], 0, 1,
                            stride=1, stride_axis=0).astype(_BF16)
            rs = [pltpu.roll(cj, (_LANES - r) % _LANES, 1) for r in range(hh)]
            zero = jnp.zeros_like(cj)
            x = jnp.concatenate(
                [jnp.where(d, r, zero) for r in rs for d in (diag0, diag1)],
                axis=1)
            w = w_block(w_ref, j).reshape(n_a, 2, hh, 2, hh, n_d)
            w = jnp.transpose(w, (2, 1, 0, 3, 4, 5))
            w = w.reshape(hh, 2, 2 * n_a, hh, n_d)
            w = jnp.concatenate(
                [w[:, 0], w[:, 1, 2 * n_a - 1:], w[:, 1, :2 * n_a - 1]], axis=1)
            part = _dot(x, w.reshape(kj, n_d))
            out = part if out is None else out + part
        return out

    issue_to(26)
    wait(x_v, S_X)
    x = x_v[0].astype(_F32)
    mu = jnp.mean(x, axis=-1, keepdims=True)
    xc = x - mu
    var = jnp.mean(xc * xc, axis=-1, keepdims=True)
    xn = (xc / jnp.sqrt(var + eps)).astype(_BF16)

    ahead = 30
    ptr = len(g0) // 2 + ahead
    issue_to(ptr)
    wait(wq_v, S_WQ)
    q = contract_major(jnp.broadcast_to(xn.astype(_F32), (n_h, n_c)),
                       wq_v).astype(_BF16)

    scale = n_d ** -0.5
    ts = []
    ptr += 14
    for j in range(n_j):
        issue_to(ptr)
        ptr += 6
        lo = j * jt + (_SHIFT_A if j else 0)
        hi = min((j + 1) * jt + _SHIFT_A, n_j * jt)
        wait(wuk_v.at[pl.ds(lo * _SUB, (hi - lo) * _SUB)], S_WUK + j)
        t = _dot_nt(q, w_block(wuk_v, j))
        ts.append(jnp.where(diag, t * scale, 0.0).astype(_BF16))
    issue_to(ptr)
    qa = _dot_nt(jnp.concatenate(ts, axis=0), e_v[...])
    q_abs = jnp.concatenate(
        [qa[j * n_h:(j + 1) * n_h] for j in range(n_j)], axis=1).astype(_BF16)

    ptr = max(ptr + 10, (len(g0) + n_ffn) // 2 + ahead)
    issue_to(ptr)
    wait(w1_v, S_W1)
    h1 = _silu(_dot_nt(xn, _untile(w1_v[...], n_j))).astype(_BF16)
    issue_to(len(pre_a))
    wait(ckv_v.at[:, pl.ds(0, _SHIFT_A)], S_KV0)

    def kv_step(i, carry):
        m, l, acc = carry

        @pl.when(i < n_main)
        def _():
            start_pairs(kv_pieces(i + _LOOK_A, 0), kv_pieces(i + _LOOK_B, 1))

        for c in range(n_main, n_blk):
            @pl.when(i == c)
            def _(c=c):
                k0 = (c - n_main) * half
                start_pairs(tail_a[k0:k0 + half], tail_b[k0:k0 + half])

        t0 = i * blk_tiles

        @pl.when(i < n_blk - 1)
        def _():
            wait(ckv_v.at[:, pl.ds(t0 + _SHIFT_A, blk_tiles)], S_KV + i)

        @pl.when(i == n_blk - 1)
        def _():
            wait(ckv_v.at[:, pl.ds(lane_tiles - blk_tiles + _SHIFT_A,
                                   blk_tiles - _SHIFT_A)], S_KV + n_blk - 1)

        kv = _untile(ckv_v[:, pl.ds(t0, blk_tiles)], n_j)
        s = _dot_nt(q_abs, kv)
        m_new = jnp.maximum(m, jnp.max(s, axis=1, keepdims=True))
        alpha = jnp.exp(m - m_new)
        p = jnp.exp(s - m_new)
        l = alpha * l + jnp.sum(p, axis=1, keepdims=True)
        acc = alpha * acc + _dot(p.astype(_BF16), kv)
        return m_new, l, acc

    m0 = jnp.full((n_h, 1), -jnp.inf, _F32)
    l0 = jnp.zeros((n_h, 1), _F32)
    a0 = jnp.zeros((n_h, n_c), _F32)
    _, l, acc = lax.fori_loop(0, n_blk, kv_step, (m0, l0, a0))
    k0 = (n_blk - n_main) * half
    start_pairs(tail_a[k0:], tail_b[k0:])
    ctx_c = acc / l

    wait(wuv_v, S_WUV)
    wait(wo_v.at[:, 0], S_WO0)
    ctx = contract_major(ctx_c, wuv_v)

    sub = 8
    row = lax.broadcasted_iota(jnp.int32, (sub, n_d), 0)
    lhs = [jnp.where(row == h % sub,
                     ctx[(h // sub) * sub:(h // sub + 1) * sub], 0.0)
           for h in range(n_h)]
    per = n_h // _N_LANE
    ctx_r = ctx.astype(_BF16).astype(_F32)
    col = {}
    for p, qq, _, _, _, _ in wo_vpu:
        h = (2 * p + 1) * per + qq
        col[p, qq] = jnp.transpose(
            jnp.broadcast_to(ctx_r[h:h + 1], (n_d, n_d)))
    a = jnp.concatenate([lhs[2 * p * per + qq] for p in range(n_pair)
                         for qq in range(per)], axis=1).astype(_BF16)
    s_v[...] = _dot(a, _untile(wo_v[:, 0], n_j))
    for qq in range(_N_WO_MXU):
        a = jnp.concatenate([lhs[(2 * p + 1) * per + qq]
                             for p in range(n_pair)], axis=1).astype(_BF16)
        lo, hi = wo_rng[qq]
        wait(wo_v.at[:, 1, pl.ds(lo, hi - lo)], S_WO + qq)
        w = wo_v[:, 1, qq * head_tiles:(qq + 1) * head_tiles]
        part = _dot(a, _untile(w, n_j)) + s_v[...]
        s_v[...] = part

    wait(w2_v, S_W2)
    g = _silu(_dot(h1, _untile(w2_v[...], n_j)))
    gb = jnp.broadcast_to(g, (sub, n_c))
    acc8 = [part[:, cb * _LANES:(cb + 1) * _LANES] for cb in range(n_j)]
    for i, (p, qq, lo, hi, t0, t1) in enumerate(wo_vpu):
        last = i == _N_WO_VPU - 1
        mult = []
        for t in range(t0, t1):
            rb, cb = divmod(t % head_tiles, n_j)
            mt = col[p, qq][rb * _SUB:(rb + 1) * _SUB]
            if last:
                mt = mt * gb[:, cb * _LANES:(cb + 1) * _LANES]
            mult.append(mt)
        if last:
            x8 = jnp.where(lax.broadcasted_iota(jnp.int32, (sub, n_c), 0) == 0,
                           jnp.broadcast_to(x, (sub, n_c)), 0.0)
            tot = jnp.concatenate(acc8, axis=1) * gb + x8
            acc8 = [tot[:, cb * _LANES:(cb + 1) * _LANES] for cb in range(n_j)]
        wait(wo_v.at[p, 1, pl.ds(lo, hi - lo)], S_WO + _N_WO_MXU + i)
        w = wo_v[p, 1, t0:t1].astype(_F32)
        terms = [[a] for a in acc8]
        for k, t in enumerate(range(t0, t1)):
            terms[t % n_j].append(w[k] * mult[k])
        acc8 = [_tree_sum(ts) for ts in terms]
    out = jnp.sum(jnp.concatenate(acc8, axis=1), axis=0, keepdims=True)
    o_ref[0] = out.astype(o_ref.dtype)


def _compiler_params():
    base = dict(vmem_limit_bytes=96 * 1024 * 1024, disable_bounds_checks=True)
    try:
        return pltpu.CompilerParams(disable_semaphore_checks=True, **base)
    except TypeError:
        return pltpu.CompilerParams(**base)


@jax.jit
def pallas_recurrent_scan__compressed_kv_cla__dense_activation_silu__decode_kernel(
    A_x: jax.Array,
    A_c_kv: jax.Array,
    A_w_q: jax.Array,
    A_w_uk: jax.Array,
    A_w_uv: jax.Array,
    A_w_o: jax.Array,
    B_x: jax.Array,
    B_w1: jax.Array,
    B_w2: jax.Array,
):
    del B_x
    b, s_q, m = A_x.shape
    _, s_k, d_c = A_c_kv.shape
    _, n_h, n_d = A_w_q.shape
    assert b == 1 and s_q == 1 and m == d_c and s_k % _KV_BLOCK == 0
    n_blk = s_k // _KV_BLOCK

    ckv = _tiles(A_c_kv.reshape(s_k, d_c)).reshape(_N_LANE, -1, _SUB, _LANES)
    wq, wuk, wuv = (w.reshape(-1, n_d) for w in (A_w_q, A_w_uk, A_w_uv))
    wo = _tiles(A_w_o.reshape(-1, m)).reshape(_N_LANE // 2, 2, -1, _SUB, _LANES)
    w1 = _tiles(B_w1.T)
    w2 = _tiles(B_w2)
    ops = (A_x, ckv, wq, wuk, wuv, wo, w1, w2)

    return pl.pallas_call(
        functools.partial(_kernel, eps=1e-5, n_h=n_h),
        in_specs=[pl.BlockSpec(memory_space=pl.ANY)] * len(ops),
        out_specs=pl.BlockSpec(memory_space=pltpu.VMEM),
        out_shape=jax.ShapeDtypeStruct(A_x.shape, A_x.dtype),
        scratch_shapes=[pltpu.VMEM(a.shape, a.dtype) for a in ops] + [
            pltpu.VMEM((_LANES, _LANES * n_h), _BF16),
            pltpu.VMEM((8, m), _F32),
            pltpu.SemaphoreType.DMA((11 + _N_WO_MXU + _N_WO_VPU + n_blk,)),
        ],
        compiler_params=_compiler_params(),
    )(*ops)
```
